```python
import os as _os
_os.environ.setdefault("JAX_PLATFORMS", "cpu")
import jax
import jax.numpy as jnp

def _softmax(x, axis=-1):
    return jax.nn.softmax(x, axis=axis)
def _gelu(x):
    return jax.nn.gelu(x, approximate=True)
def _silu(x):
    return jax.nn.silu(x)
def _sigmoid(x):
    return jax.nn.sigmoid(x)
def _layernorm(x, axis=-1, eps=1e-5):
    m = jnp.mean(x, axis=axis, keepdims=True)
    v = jnp.var(x, axis=axis, keepdims=True)
    return (x - m) / jnp.sqrt(v + eps)
def _scatter_add(tgt, idx, src, axis=0):
    return tgt.at[idx].add(src)
def _segment_sum(src, seg, n):
    return jax.ops.segment_sum(src, seg, n)
class _Rng:
    def __init__(self, key):
        self._k = key
    def _next(self):
        self._k, sub = jax.random.split(self._k)
        return sub
    def normal(self, shape):
        return jax.random.normal(self._next(), shape, dtype=jnp.bfloat16)
    def randint(self, lo, hi, shape):
        return jax.random.randint(self._next(), shape, lo, hi, dtype=jnp.int32)
    def uniform(self, shape, lo=0.0, hi=1.0):
        return jax.random.uniform(self._next(), shape, jnp.bfloat16, lo, hi)
    def permutation(self, n):
        return jax.random.permutation(self._next(), n)


kernel_name = 'interleave_layers__spectral_gfnet__mixer_token_mlp__prompt'

def setup_inputs():
    _rng = _Rng(jax.random.key(int.from_bytes(__import__("os").urandom(4), "little")))
    _w = (lambda a: (lambda t: t.astype(jnp.bfloat16) if jnp.issubdtype(t.dtype, jnp.floating) else t)(jnp.asarray(a)))
    def _A_setup():
        B, S, D = 1, 2048, 640
        Df = D // 2 + 1
        return {
            "x": _w((lambda *s: _rng.normal(s) * 0.05)(B, S, D)),
            "w_r": _w((lambda *s: _rng.normal(s) * 0.2)(S, Df) * 0.02),
            "w_i": _w((lambda *s: _rng.normal(s) * 0.2)(S, Df) * 0.02),
        }
    _A_in = _A_setup()

    def _B_setup():
        B, S, D, F = 1, 2048, 640, 1728
        return {
            "x": _w((lambda *s: _rng.normal(s) * 0.05)(B, S, D)),
            "w1": _w((lambda *s: _rng.normal(s) * 0.1)(S, F) * (S ** -0.5)),
            "b1": _w((lambda *s: _rng.normal(s) * 0.1)(F) * 0.02),
            "w2": _w((lambda *s: _rng.normal(s) * 0.1)(F, S) * (F ** -0.5)),
            "b2": _w((lambda *s: _rng.normal(s) * 0.1)(S) * 0.02),
        }
    _B_in = _B_setup()

    return {
        "A_x": _A_in["x"],
        "A_w_r": _A_in["w_r"],
        "A_w_i": _A_in["w_i"],
        "B_x": _B_in["x"],
        "B_w1": _B_in["w1"],
        "B_b1": _B_in["b1"],
        "B_w2": _B_in["w2"],
        "B_b2": _B_in["b2"],
    }

def reference(A_x, A_w_r, A_w_i, B_x, B_w1, B_b1, B_w2, B_b2):
    def _A_ref(x, w_r, w_i):
        B, S, D = x.shape
        X = (lambda x, axes=(-2,-1): jnp.fft.rfft2(x.astype(jnp.float32), axes=axes))(x, axes=(-2, -1))
        W = w_r + 1j * w_i
        X = X * W
        y = (lambda x, s, axes=(-2,-1): jnp.fft.irfft2(x, s=s, axes=axes).astype(jnp.bfloat16))(X, (S, D), axes=(-2, -1))
        return y

    def _B_ref(x, w1, b1, w2, b2):
        B, S, D = x.shape
        h = _layernorm(x, axis=-1)
        u = jnp.einsum("bsd,sf->bdf", h, w1) + b1
        u = _gelu(u)
        y = jnp.einsum("bdf,fs->bds", u, w2) + b2
        return (lambda x, *d: x.transpose(*d))(y, 0, 2, 1)

    x = A_x
    x = x + _A_ref(_layernorm(x, axis=-1), A_w_r, A_w_i)
    x = x + _B_ref(_layernorm(x, axis=-1), B_w1, B_b1, B_w2, B_b2)
    x = x + _A_ref(_layernorm(x, axis=-1), A_w_r, A_w_i)
    x = x + _B_ref(_layernorm(x, axis=-1), B_w1, B_b1, B_w2, B_b2)
    return x
```

```python
import contextlib
import functools
import itertools
import math

import jax
import jax.numpy as jnp
import jax.experimental.pallas as pl
import jax.experimental.pallas.tpu as pltpu

S = 2048
D = 640
DF = D // 2 + 1
F = 1728
R = 336
EPS = 1e-5
CW = 256
NCH = S // CW
F32 = jnp.float32
BF16 = jnp.bfloat16
NT = (((1,), (1,)), ((), ()))

_C1, _C2 = math.cos(2 * math.pi / 5), math.cos(4 * math.pi / 5)
_S1, _S2 = math.sin(2 * math.pi / 5), math.sin(4 * math.pi / 5)
_KN = (_C1 - _C2) / 2
_RES = ((0, 5), (1, 9), (2, 8), (3, 7), (4, 6))
_BASE = (None, 9, 2, 7, 4)
_SC = (None, _S2, _S1, _S1, _S2)


def _dft5(a):
    a1 = a[1] + a[4]
    b1 = a[1] - a[4]
    a2 = a[2] + a[3]
    b2 = a[2] - a[3]
    t = a1 + a2
    y0 = a[0] + t
    m = a[0] - 0.25 * t
    n = _KN * (a1 - a2)
    return y0, m + n, b1 + (_S2 / _S1) * b2, m - n, b1 - (_S1 / _S2) * b2


def _dft5_t(y0, y1r, y1i, y2r, y2i):
    gm = y1r + y2r
    gn = _KN * (y1r - y2r)
    a0 = y0 + gm
    gt = y0 - 0.25 * gm
    ga1 = gt + gn
    ga2 = gt - gn
    gb1 = y1i + y2i
    gb2 = (_S2 / _S1) * y1i - (_S1 / _S2) * y2i
    return [a0, ga1 + gb1, ga2 + gb2, ga2 - gb2, ga1 - gb1]


def _dft4(x, sign):
    (ar, ai), (br, bi), (cr, ci), (dr, di) = x
    t0r, t0i = ar + cr, ai + ci
    t1r, t1i = ar - cr, ai - ci
    t2r, t2i = br + dr, bi + di
    t3r, t3i = br - dr, bi - di
    y0 = (t0r + t2r, t0i + t2i)
    y2 = (t0r - t2r, t0i - t2i)
    if sign < 0:
        y1 = (t1r + t3i, t1i - t3r)
        y3 = (t1r - t3i, t1i + t3r)
    else:
        y1 = (t1r - t3i, t1i + t3r)
        y3 = (t1r + t3i, t1i - t3r)
    return [y0, y1, y2, y3]


def _twid16(v, e, sign):
    r, i = v
    e = e % 16
    if e == 0:
        return v
    h = math.sqrt(0.5)
    if e == 4:
        return (-i, r) if sign > 0 else (i, -r)
    if e == 2:
        return (h * (r - i), h * (r + i)) if sign > 0 else (h * (r + i), h * (i - r))
    if e == 6:
        return (-h * (r + i), h * (r - i)) if sign > 0 else (h * (i - r), -h * (r + i))
    c = math.cos(2 * math.pi * e / 16)
    s = sign * math.sin(2 * math.pi * e / 16)
    return (c * r - s * i, s * r + c * i)


def _iota(shape, dim):
    return jax.lax.broadcasted_iota(jnp.int32, shape, dim)


def _cos_quarter(t):
    q = jnp.floor(t + 0.5)
    x = (t - q) * (math.pi / 2)
    x2 = x * x
    c = 1.0 + x2 * (-1.0 / 2 + x2 * (1.0 / 24 + x2 * (-1.0 / 720 + x2 * (1.0 / 40320))))
    s = x * (1.0 + x2 * (-1.0 / 6 + x2 * (1.0 / 120 + x2 * (-1.0 / 5040 + x2 * (1.0 / 362880)))))
    qi = q.astype(jnp.int32)
    v = jnp.where((qi & 1) == 1, s, c)
    return jnp.where(((qi + 1) & 2) == 2, -v, v)


_ROWS = (80, 64, 64, 64, 64)
W1C = 256
NW1 = -(-F // W1C)
W2C = 216
NW2 = F // W2C
NFT = -(-F // 128)
NT_ = S // 128
TPC = CW // 128
U32 = jnp.uint32
NZ = 16


def _dot(a, b):
    return jnp.dot(a, b, preferred_element_type=F32)


def _tile(n):
    return slice(128 * n, 128 * n + 128)


def _weave(*streams):
    live = [[g, n, 0] for g, n in streams if g is not None]
    while live:
        cur = min(live, key=lambda e: (e[2] + 0.5) / e[1])
        try:
            next(cur[0])
            cur[2] += 1
        except StopIteration:
            live.remove(cur)


def _scratch():
    v = lambda shape, dt: pltpu.VMEM((1,) + shape, dt)
    return dict(
        xio=pltpu.VMEM((S, D), BF16),
        wraw=pltpu.VMEM((640, S), BF16),
        wlast=pltpu.VMEM((2, 1, S), BF16),
        w1t=pltpu.VMEM((F, S), BF16),
        w2=pltpu.VMEM((F, S), BF16),
        wt1=[v((S // 2, 128), U32) for _ in range(5)],
        wt2=v((8, 640, 128), U32),
        wex=v((16, 2, 8, 128), F32),
        ACC=[v((128, W1C), F32) for _ in range(5)],
        XA=[v((D, 128), F32) for _ in range(NT_)],
        XB=[v((D, 128), F32) for _ in range(NT_)],
        YB=[v((5, 128, 128), BF16) for _ in range(NT_)],
        Z=[v((2, r, S), F32) for r in _ROWS],
        U=[v((2, r, S), F32) for r in _ROWS],
        XS=[v((2, r, S), F32) for r in _ROWS],
        V=[v((2, r, S), F32) for r in _ROWS],
        Q=[[v((4, 128, 128), F32) for _ in range(4)] for _ in range(5)],
        HB=[v((D, 128), BF16) for _ in range(NT_)],
        GB=[v((D, 128), BF16) for _ in range(NFT)],
        gf=v((16, 3, 128, 128), BF16),
        gi=v((16, 3, 128, 128), BF16),
        mf=v((5, 144, 128), BF16),
        mi=v((5, 128, 128), BF16),
        sem_x=pltpu.SemaphoreType.DMA((NCH,)),
        sem_w=pltpu.SemaphoreType.DMA((8,)),
        sem_w1=pltpu.SemaphoreType.DMA((NW1,)),
        sem_w2=pltpu.SemaphoreType.DMA((NW2,)),
        sem_o=pltpu.SemaphoreType.DMA((NCH,)),
        sem_z=pltpu.SemaphoreType.REGULAR,
        sem_f=pltpu.SemaphoreType.REGULAR,
    )


def _kernel(x_hbm, wr_hbm, wi_hbm, w1t_hbm, b1_ref, w2_hbm, b2_ref, o_hbm, *scratch):
    sc = jax.tree_util.tree_unflatten(jax.tree_util.tree_structure(_scratch(), is_leaf=_is_leaf), scratch)
    xio, wraw, wlast, w1t, w2 = sc["xio"], sc["wraw"], sc["wlast"], sc["w1t"], sc["w2"]
    wt1, wt2, XA, XB, YB, Z, U, XS, V, Q = (sc[k] for k in ("wt1", "wt2", "XA", "XB", "YB", "Z", "U", "XS", "V", "Q"))
    wex, ACC = sc["wex"], sc["ACC"]
    HB, GB, gf, gi, mf, mi = (sc[k] for k in ("HB", "GB", "gf", "gi", "mf", "mi"))
    sem_x, sem_w, sem_w1, sem_w2, sem_o = (sc[k] for k in ("sem_x", "sem_w", "sem_w1", "sem_w2", "sem_o"))

    zpool = [pl.semaphore_read(sc["sem_z"]) for _ in range(NZ)]
    lay = [0]

    def zz(i=0):
        return zpool[8 * lay[0] + i]

    def ldb(ref, z, *idx):
        return pltpu.bitcast(ref.bitcast(U32)[(z,) + idx], BF16)

    def x_copy(c):
        return pltpu.make_async_copy(x_hbm.at[0, pl.ds(c * CW, CW), :], xio.at[pl.ds(c * CW, CW), :], sem_x.at[c])

    def o_copy(c):
        return pltpu.make_async_copy(xio.at[pl.ds(c * CW, CW), :], o_hbm.at[0, pl.ds(c * CW, CW), :], sem_o.at[c])

    w_parts = [[(wr_hbm, 0, 0, 128)], [(wr_hbm, 128, 128, 128)], [(wr_hbm, 256, 256, 64), (wi_hbm, 0, 320, 64)],
               [(wi_hbm, 64, 384, 128)], [(wi_hbm, 192, 512, 128)]]
    w_copies, n = [], 0
    for blk in w_parts:
        cur = []
        for (src, s0, d0, rows) in blk:
            cur.append(pltpu.make_async_copy(src.at[pl.ds(s0, rows), :], wraw.at[pl.ds(d0, rows), :], sem_w.at[n]))
            n += 1
        w_copies.append(cur)
    for a, src in enumerate((wr_hbm, wi_hbm)):
        w_copies[0].insert(0, pltpu.make_async_copy(src.at[pl.ds(320, 1), :], wlast.at[a], sem_w.at[n]))
        n += 1

    def w1_copy(i):
        rows = min(W1C, F - i * W1C)
        return pltpu.make_async_copy(w1t_hbm.at[pl.ds(i * W1C, rows), :], w1t.at[pl.ds(i * W1C, rows), :], sem_w1.at[i])

    def w2_copy(i):
        return pltpu.make_async_copy(w2_hbm.at[pl.ds(i * W2C, W2C), :], w2.at[pl.ds(i * W2C, W2C), :], sem_w2.at[i])

    for c in range(NCH):
        x_copy(c).start()
    for blk in w_copies:
        for cp in blk:
            cp.start()

    def d_tables():
        row = _iota((128, 128), 0)
        col = _iota((128, 128), 1)
        n2 = col & 63
        is_b = col >= 64
        is_im = (row & 8) == 8
        rr = ((row >> 4) << 3) | (row & 7)
        j = rr & 31
        second = rr >= 32
        for g in range(5):
            ra, rb = _RES[g]
            kb = jnp.where(second, rb, ra) + 10 * j
            idx = kb * n2
            if g == 0:
                idx = idx + jnp.where(is_im, 160, 0)
                amp = jnp.where(second == is_b, 1.0, 0.0).astype(F32)
            else:
                idx = idx + jnp.where(is_im != is_b, 160, 0)
                sg = jnp.where((rb == _BASE[g]) == second, 1.0, -1.0).astype(F32)
                amp = jnp.where(is_b, jnp.where(is_im, -sg * _SC[g], sg * _SC[g]), 1.0).astype(F32)
            m = amp * _cos_quarter(idx.astype(F32) * (1.0 / 160))
            mf[0, g, 0:128, :] = m.astype(BF16)
            mt = m * (2.0 / (S * D))
            if g == 0:
                mt = jnp.where(kb == 0, 0.5 * mt, mt)
                nyq = jnp.where(is_b, 0.0, jnp.where((n2 & 1) == 0, 1.0, -1.0)).astype(F32)
                mt = jnp.where(row == 8, nyq * (1.0 / (S * D)), mt)
                r16 = _iota((16, 128), 0)
                c16 = _iota((16, 128), 1)
                ext = jnp.where((r16 == 0) & (c16 < 64), jnp.where((c16 & 1) == 0, 1.0, -1.0), 0.0).astype(F32)
                mf[0, 0, 128:144, :] = ext.astype(BF16)
            mi[0, g] = mt.T.astype(BF16)

    def s_tables(which):
        tab = (gf, gi)[which]
        for i in range(8):
            row = _iota((16, 128), 0) + 16 * i
            col = _iota((16, 128), 1)
            n2, l = (row, col) if which == 0 else (col, row)
            k2 = 8 * (l & 15) + (l >> 4)
            t0 = ((n2 * k2) & 127).astype(F32) * (1.0 / 32)
            ga = _cos_quarter(t0)
            gb = _cos_quarter(t0 + 1.0)
            t1 = n2.astype(F32) * (1.0 / 512)
            ta = _cos_quarter(t1)
            tb = _cos_quarter(t1 + 1.0)
            rs = slice(16 * i, 16 * i + 16)
            for k1 in range(16):
                tab[0, k1, 0, rs, :] = ga.astype(BF16)
                tab[0, k1, 1, rs, :] = (gb - ga).astype(BF16)
                tab[0, k1, 2, rs, :] = (ga + gb).astype(BF16)
                if k1 < 15:
                    ga, gb = ga * ta - gb * tb, ga * tb + gb * ta
                if k1 % 8 == 7:
                    yield

    ctiles = lambda c: list(range(TPC * c, TPC * (c + 1)))

    def x_in(c):
        for t in range(TPC * c, TPC * (c + 1)):
            for j in range(5):
                XA[t][0, _tile(j), :] = xio[_tile(t), _tile(j)].T.astype(F32)
                yield

    rstd, mean = {}, {}

    def front_vpu(tiles):
        for t in tiles:
            z = zz()
            e0s, ssq = [], None
            for rp in range(4):
                xs = [XA[t][z, 64 * n + 16 * rp: 64 * n + 16 * rp + 16, :] for n in range(10)]
                sm = [xs[n] + xs[n + 5] for n in range(5)]
                df = [xs[n] - xs[n + 5] if n % 2 == 0 else xs[n + 5] - xs[n] for n in range(5)]
                e0, e1r, e1i, e2r, e2i = _dft5(sm)
                o0, o1r, o1i, o2r, o2i = _dft5(df)
                q = (0.5 * (o0 * o0) + (e1r * e1r + e2r * e2r + o1r * o1r + o2r * o2r)
                     + (_S1 * _S1) * (e1i * e1i + o1i * o1i) + (_S2 * _S2) * (e2i * e2i + o2i * o2i))
                ssq = q if ssq is None else ssq + q
                e0s.append(e0)
                a, b = slice(16 * rp, 16 * rp + 16), slice(64 + 16 * rp, 64 + 16 * rp + 16)
                YB[t][0, 0, b, :] = o0.astype(BF16)
                for g, (va, vb) in enumerate(((o2r, o2i), (e1r, e1i), (o1r, o1i), (e2r, e2i))):
                    YB[t][0, g + 1, a, :] = va.astype(BF16)
                    YB[t][0, g + 1, b, :] = vb.astype(BF16)
                if rp < 3:
                    yield
            tot = jnp.sum(e0s[0] + e0s[1] + e0s[2] + e0s[3], axis=0, keepdims=True)
            mu10 = tot * (1.0 / 64)
            mean[t] = tot * (1.0 / D)
            e0s = [e - mu10 for e in e0s]
            q0 = e0s[0] * e0s[0] + e0s[1] * e0s[1] + e0s[2] * e0s[2] + e0s[3] * e0s[3]
            var = jnp.sum(ssq + 0.5 * q0, axis=0, keepdims=True) * (2.0 / (10 * D))
            rstd[t] = jax.lax.rsqrt(var + EPS)
            for rp in range(4):
                YB[t][0, 0, 16 * rp: 16 * rp + 16, :] = e0s[rp].astype(BF16)
            yield

    def front_mxu(tiles):
        z = zz(tiles[0] // TPC)
        for g in range(5):
            lhs = ldb(mf, z, 0) if g == 0 else ldb(mf, z, g, slice(0, 64))
            for t in tiles:
                y = _dot(lhs, ldb(YB[t], z, g)) * rstd[t]
                for i in range(8):
                    for p in range(2):
                        Z[g][0, p, 8 * i: 8 * i + 8, _tile(t)] = y[16 * i + 8 * p: 16 * i + 8 * p + 8]
                if g == 0:
                    Z[0][0, 0, 64:72, _tile(t)] = y[128:136]
            yield

    def ld(src, z, rs, n):
        return (src[z, 0, rs, _tile(n)], src[z, 1, rs, _tile(n)])

    def st(dst, rs, n, v):
        dst[0, 0, rs, _tile(n)] = v[0]
        dst[0, 1, rs, _tile(n)] = v[1]

    def stage_a(g):
        z = zz()
        for i in range(9 if g == 0 else 8):
            rs = slice(8 * i, 8 * i + 8)
            for b in range(4):
                t = _dft4([ld(Z[g], z, rs, 4 * a + b) for a in range(4)], -1)
                for ka in range(4):
                    st(U[g], rs, 4 * ka + b, _twid16(t[ka], b * ka, -1))
            yield

    def pass_f(g):
        rs = slice(0, _ROWS[g])
        for ka in range(4):
            for par in range(2):
                z = zz(par)
                zt = zz(g)
                (ar, ai), (br, bi), (cr, ci), (dr, di) = [ld(U[g], z, rs, 4 * ka + b) for b in range(4)]
                if par == 0:
                    t0r, t0i, t2r, t2i = ar + cr, ai + ci, br + dr, bi + di
                    outs = [(t0r + t2r, t0i + t2i), (t0r - t2r, t0i - t2i)]
                else:
                    t1r, t1i, t3r, t3i = ar - cr, ai - ci, br - dr, bi - di
                    outs = [(t1r + t3i, t1i - t3r), (t1r - t3i, t1i + t3r)]
                for h, (ur, ui) in enumerate(outs):
                    k1 = ka + 4 * (par + 2 * h)
                    p1 = _dot((ur + ui).astype(BF16), ldb(gf, zt, k1, 0))
                    p2 = _dot(ur.astype(BF16), ldb(gf, zt, k1, 1))
                    p3 = _dot(ui.astype(BF16), ldb(gf, zt, k1, 2))
                    st(XS[g], rs, k1, (p1 - p3, p1 + p2))
                yield

    def w_rows(z, a, g, k1):
        parts = []
        for res in _RES[g]:
            blk = wt2[z, k1 // 2, pl.ds(320 * a + res, 32, stride=10), :]
            blk = (blk << 16) if k1 % 2 == 0 else (blk & jnp.uint32(0xFFFF0000))
            parts.append(pltpu.bitcast(blk, F32))
        if g == 0:
            parts.append(wex[z, k1, a])
            parts.append(jnp.zeros((8, 128), F32))
        return jnp.concatenate(parts, axis=0)

    def pass_i(g):
        rs = slice(0, _ROWS[g])
        z = zz(g)
        for ka in range(4):
            vs = []
            for kb in range(4):
                k1 = ka + 4 * kb
                xr, xi = ld(XS[g], z, rs, k1)
                wr = w_rows(z, 0, g, k1)
                wi = w_rows(z, 1, g, k1)
                yr = xr * wr - xi * wi
                yi = xr * wi + xi * wr
                q1 = _dot((yr + yi).astype(BF16), ldb(gi, z, k1, 0))
                q2 = _dot(yi.astype(BF16), ldb(gi, z, k1, 1))
                q3 = _dot(yr.astype(BF16), ldb(gi, z, k1, 2))
                vs.append((q1 + q2, q1 - q3))
                if kb % 2 == 1 and kb < 3:
                    yield
            t = _dft4(vs, +1)
            for b in range(4):
                st(V[g], rs, 4 * ka + b, _twid16(t[b], b * ka, +1))
            yield

    def pass_b(g, bs=range(4)):
        for b in bs:
            z = zz(b)
            rhs = [[] for _ in range(4)]
            for i in range(8):
                rs = slice(8 * i, 8 * i + 8)
                y = _dft4([ld(V[g], z, rs, 4 * ka + b) for ka in range(4)], +1)
                if g == 0 and i == 0:
                    r8 = _iota((8, 128), 0)
                    ex = _dft4([ld(V[0], z, slice(64, 72), 4 * ka + b) for ka in range(4)], +1)
                    y = [(y[a][0], jnp.where(r8 == 0, ex[a][0], y[a][1])) for a in range(4)]
                for a in range(4):
                    rhs[a] += [y[a][0], y[a][1]]
            yield
            for a in range(4):
                Q[g][b][0, a] = _dot(ldb(mi, z, g), jnp.concatenate(rhs[a], axis=0).astype(BF16))
            yield

    def s_round(ga, gf_, gi_, gb_, *extra):
        ok = lambda g: g is not None and 0 <= g < 5
        _weave((stage_a(ga) if ok(ga) else None, 8), (pass_f(gf_) if ok(gf_) else None, 8),
               (pass_i(gi_) if ok(gi_) else None, 8), (pass_b(gb_) if ok(gb_) else None, 8), *extra)

    def back_vpu(tiles):
        for t in tiles:
            z = zz()
            z = zz(1)
            qa, qb = t // 4, t % 4
            q = lambda g, rs: Q[g][qb][z, qa, rs, :]
            q0 = [q(0, slice(8 * rp, 8 * rp + 8)) for rp in range(8)]
            qs = ((q0[0] + q0[1]) + (q0[2] + q0[3])) + ((q0[4] + q0[5]) + (q0[6] + q0[7]))
            mu = mean[t] + jnp.sum(qs, axis=0, keepdims=True) * (10.0 / D)
            mean[t] = mu
            s2 = [None, None]
            for rp in range(8):
                a, b = slice(8 * rp, 8 * rp + 8), slice(64 + 8 * rp, 64 + 8 * rp + 8)
                e = _dft5_t(q0[rp] - mu, q(2, a), q(2, b), q(4, a), q(4, b))
                o = _dft5_t(q(0, b), q(3, a), q(3, b), q(1, a), q(1, b))
                for n in range(5):
                    lo = slice(64 * n + 8 * rp, 64 * n + 8 * rp + 8)
                    hi = slice(64 * (n + 5) + 8 * rp, 64 * (n + 5) + 8 * rp + 8)
                    if n % 2 == 0:
                        ylo, yhi = e[n] + o[n], e[n] - o[n]
                    else:
                        ylo, yhi = e[n] - o[n], e[n] + o[n]
                    xlo = XA[t][z, lo, :] + ylo
                    xhi = XA[t][z, hi, :] + yhi
                    XB[t][0, lo, :] = xlo
                    XB[t][0, hi, :] = xhi
                    s2[0] = xlo * xlo if s2[0] is None else s2[0] + xlo * xlo
                    s2[1] = xhi * xhi if s2[1] is None else s2[1] + xhi * xhi
                if rp % 2 == 1:
                    yield
            var = jnp.sum(s2[0] + s2[1], axis=0, keepdims=True) * (1.0 / D)
            r1 = jax.lax.rsqrt(var + EPS)
            r2 = jax.lax.rsqrt(var * r1 * r1 + EPS)
            rr = r1 * r2
            for i in range(D // 16):
                HB[t][0, 16 * i: 16 * i + 16, :] = (XB[t][z, 16 * i: 16 * i + 16, :] * rr).astype(BF16)
            yield

    b1 = b1_ref[...].astype(F32).reshape(1, F)
    b2 = b2_ref[...].astype(F32).reshape(1, S)

    def act(u, off, w):
        g = jax.nn.gelu(u + b1[:, off: off + w], approximate=True).astype(BF16)
        for j in range(0, w, 128):
            ww = min(128, w - j)
            GB[(off + j) // 128][0, :, 0:ww] = g[:, j: j + ww]

    def mm1_dot(off, w, tiles):
        z = zz(off // W1C)
        lhs = jnp.concatenate([ldb(HB[t], z) for t in tiles], axis=1)
        rhs = jnp.concatenate([w1t[off: off + w, _tile(t)] for t in tiles], axis=1)
        return jax.lax.dot_general(lhs, rhs, NT, preferred_element_type=F32)

    def mm1_step(tiles, first):
        z = zz()
        rhs = jnp.concatenate([w1t[0:W1C, _tile(t)] for t in tiles], axis=1)
        for rb in range(5):
            lhs = jnp.concatenate([ldb(HB[t], z, slice(64 * rb, 64 * rb + 64)) for t in tiles], axis=1)
            part = jax.lax.dot_general(lhs, rhs, NT, preferred_element_type=F32)
            ACC[rb][0] = part if first else ACC[rb][z] + part
            yield

    def mm2(c):
        z = zz(c)
        cs = slice(c * CW, (c + 1) * CW)
        parts = [ldb(GB[j], z) for j in range(NFT - 1)] + [ldb(GB[NFT - 1], z, slice(None), slice(0, F % 128))]
        y = _dot(jnp.concatenate(parts, axis=1), w2[:, cs])
        return [XB[t][zz(2)] + (y[:, _tile(i)] + (b2[:, _tile(t)] + mean[t])) for i, t in enumerate(ctiles(c))]

    def w_prep(b):
        for jt in range(16):
            blk = pltpu.bitcast(wraw[_tile(b), _tile(jt)].T, U32)
            for a in range(8):
                pos = 8 * (16 * a + jt)
                wt1[b][0, pos: pos + 8, :] = blk[8 * a: 8 * a + 8]
            yield
        z = zz()
        for m in range(8):
            wt2[0, m, _tile(b), :] = wt1[b][z, pl.ds(m, 128, stride=8), :].T
            yield

    def w_extra():
        r8 = _iota((8, S), 0)
        lane = _iota((8, 128), 1)
        e = jnp.where(r8 == 0, jnp.broadcast_to(wlast[0].astype(F32), (8, S)),
                      jnp.where(r8 == 1, jnp.broadcast_to(wlast[1].astype(F32), (8, S)), 0.0))
        v = [e[:, _tile(n)] for n in range(16)]
        for b in range(4):
            stp = 1 << b
            msk = (lane & stp) == 0
            for n in range(16):
                if n & stp:
                    continue
                lo, hi = v[n], v[n | stp]
                v[n] = jnp.where(msk, lo, pltpu.roll(hi, stp, 1))
                v[n | stp] = jnp.where(msk, pltpu.roll(lo, 128 - stp, 1), hi)
            yield
        r = _iota((8, 128), 0)
        for n in range(16):
            wex[0, n, 0] = jnp.where(r == 0, v[n], 0.0)
            wex[0, n, 1] = jnp.where(r == 0, pltpu.roll(v[n], 7, 0), 0.0)
        yield

    def scope(name):
        return contextlib.nullcontext()

    def fence():
        pl.semaphore_signal(sc["sem_f"], 1)
        pl.semaphore_wait(sc["sem_f"], 1)

    with scope("p0_tables"):
        d_tables()
        Z[0][0, 1, 64:72, :] = jnp.zeros((8, S), F32)
        U[0][0, :, 72:80, :] = jnp.zeros((2, 8, S), F32)
    tf = s_tables(0)
    with scope("p1_front"):
        for c in range(NCH + 2):
            if c < NCH:
                x_copy(c).wait()
            _weave((x_in(c) if c < NCH else None, 5 * TPC),
                   (front_vpu(ctiles(c - 1)) if 0 <= c - 1 < NCH else None, 4 * TPC),
                   (front_mxu(ctiles(c - 2)) if 0 <= c - 2 < NCH else None, 5),
                   (itertools.islice(tf, 2), 2))
    ti = s_tables(1)
    for layer in range(2):
        lay[0] = layer
        if layer == 0:
            wq = {0: (0, 1), 3: (2, 3), 5: (4,)}
            wn = (8, 22, 18, 24, 24, 24)
            with scope("p2_F0"):
                for r in range(6):
                    extra = [(itertools.islice(ti, 3), 3)] if r > 0 else []
                    if r in wq:
                        if r == 5:
                            for i in range(3):
                                w1_copy(i).start()
                        for bb in wq[r]:
                            for cp in w_copies[bb]:
                                cp.wait()
                        wp = itertools.chain(*[w_prep(bb) for bb in wq[r]])
                    if r == 1:
                        extra.append((w_extra(), 5))
                    if r == 5:
                        extra.append((ti, 1))
                    extra.append((itertools.islice(wp, wn[r]), wn[r]))
                    s_round(r, r - 1, None, None, *extra)
            with scope("p3_I0"):
                for r in range(5):
                    s_round(None, None, r, r - 1)
                for i in range(3, NW1):
                    w1_copy(i).start()
                for i in range(3):
                    w1_copy(i).wait()
        else:
            with scope("q2_S1"):
                for r in range(7):
                    s_round(r, r - 1, r - 2, r - 3)
                fence()
        pairs = [(b + 8 * hh, b + 8 * hh + 4) for b in range(4) for hh in range(2)]
        with scope("p4_back%d" % layer):
            _weave((pass_b(4, [0]), 2))
            for i in range(len(pairs) + 1):
                _weave((pass_b(4, [1, 2, 3]) if i == 0 else None, 6),
                       (back_vpu(pairs[i]) if i < len(pairs) else None, 10),
                       (mm1_step(pairs[i - 1], i == 1) if i >= 1 else None, 5))
            if layer == 0:
                for i in range(NW2):
                    w2_copy(i).start()
                for i in range(3, NW1):
                    w1_copy(i).wait()
            else:
                fence()
        with scope("p5_mm_%d" % layer):
            z = zz()
            acc = jnp.concatenate([ACC[rb][z] for rb in range(5)], axis=0)
            pend = (acc, 0, W1C)
            for i in range(1, NW1):
                if layer == 0 and i == NW1 - 1:
                    for ii in range(NW2):
                        w2_copy(ii).wait()
                off = i * W1C
                w = min(W1C, F - off)
                cur = (mm1_dot(off, w, range(NT_)), off, w)
                act(*pend)
                pend = cur
            act(*pend)
            for c in range(NCH + 1):
                if c < NCH:
                    xn = mm2(c)
                if layer == 0:
                    if c < NCH:
                        for t, v in zip(ctiles(c), xn):
                            XA[t][0] = v
                    if c >= 1:
                        lay[0] = 1
                        _weave((front_vpu(ctiles(c - 1)), 8))
                        _weave((front_mxu(ctiles(c - 1)), 5))
                        lay[0] = 0
                else:
                    if c >= 1:
                        for t, v in zip(ctiles(c - 1), xprev):
                            xio[_tile(t), :] = v.astype(BF16).T
                        o_copy(c - 1).start()
                        if c in (4, 6, 7):
                            fence()
                    xprev = xn
            if layer == 0:
                fence()

    with scope("p7_out"):
        for c in range(NCH):
            o_copy(c).wait()


def _is_leaf(x):
    return not isinstance(x, (dict, list))


@jax.jit
def pallas_interleave_layers__spectral_gfnet__mixer_token_mlp__prompt_kernel(A_x, A_w_r, A_w_i, B_x, B_w1, B_b1, B_w2, B_b2):
    del B_x
    any_spec = pl.BlockSpec(memory_space=pl.ANY)
    vmem_spec = pl.BlockSpec(memory_space=pltpu.VMEM)
    return pl.pallas_call(
        _kernel,
        out_shape=jax.ShapeDtypeStruct((1, S, D), BF16),
        in_specs=[any_spec, any_spec, any_spec, any_spec, vmem_spec, any_spec, vmem_spec],
        out_specs=any_spec,
        scratch_shapes=jax.tree_util.tree_leaves(_scratch(), is_leaf=_is_leaf),
        compiler_params=pltpu.CompilerParams(vmem_limit_bytes=120 * 1024 * 1024),
    )(A_x, A_w_r.T, A_w_i.T, B_w1.T, B_b1, B_w2, B_b2)
```

```python
import contextlib
import itertools
import math

import jax
import jax.numpy as jnp
import jax.experimental.pallas as pl
import jax.experimental.pallas.tpu as pltpu

S = 2048
D = 640
F = 1728
EPS = 1e-5
F32 = jnp.float32
BF16 = jnp.bfloat16
U32 = jnp.uint32
NT = (((1,), (1,)), ((), ()))

_C1, _C2 = math.cos(2 * math.pi / 5), math.cos(4 * math.pi / 5)
_S1, _S2 = math.sin(2 * math.pi / 5), math.sin(4 * math.pi / 5)
_KN = (_C1 - _C2) / 2
_RES = ((0, 5), (1, 9), (2, 8), (3, 7), (4, 6))
_BASE = (None, 9, 2, 7, 4)
_SC = (None, _S2, _S1, _S1, _S2)
_ROWS = (80, 64, 64, 64, 64)

W1C = 384
NW1 = -(-F // W1C)
W2C = 216
NW2 = F // W2C
NFT = -(-F // 128)
NTT = S // 128
NZ = 16
MIR = 64
STOP = ''
STEP4 = 1
FENCES = 'ac'
W1S = [int(x) for x in '384,384,384,192'.split(',')]
DS = 512
_PAIRS = [(b + 8 * h, b + 8 * h + 4) for b in range(4) for h in range(2)]
_XSEG = [[[0, 4, 8, 12], [1, 5, 9, 13], [2, 6, 10, 14], [3, 7, 11, 15]],
         [[0, 4, 8, 12], [1, 5, 9, 13], [2, 6, 10, 14], [3, 7, 11], [15]],
         [[0, 4], [8, 12, 1, 5], [9, 13, 2, 6], [10, 14, 3, 7], [11, 15]],
         [[0, 4, 8, 12], [1, 5, 9, 13], [2, 6], [10, 14], [3, 7], [11, 15]]][3]
LAG = 1
XMXU = 0


def _dft5(a):
    a1 = a[1] + a[4]
    b1 = a[1] - a[4]
    a2 = a[2] + a[3]
    b2 = a[2] - a[3]
    t = a1 + a2
    y0 = a[0] + t
    m = a[0] - 0.25 * t
    n = _KN * (a1 - a2)
    return y0, m + n, b1 + (_S2 / _S1) * b2, m - n, b1 - (_S1 / _S2) * b2


def _dft5_t(y0, y1r, y1i, y2r, y2i):
    gm = y1r + y2r
    gn = _KN * (y1r - y2r)
    a0 = y0 + gm
    gt = y0 - 0.25 * gm
    ga1 = gt + gn
    ga2 = gt - gn
    gb1 = y1i + y2i
    gb2 = (_S2 / _S1) * y1i - (_S1 / _S2) * y2i
    return [a0, ga1 + gb1, ga2 + gb2, ga2 - gb2, ga1 - gb1]


def _dft4_half(x, sign, par):
    (ar, ai), (br, bi), (cr, ci), (dr, di) = x
    if par == 0:
        t0r, t0i, t2r, t2i = ar + cr, ai + ci, br + dr, bi + di
        return [(t0r + t2r, t0i + t2i), (t0r - t2r, t0i - t2i)]
    t1r, t1i, t3r, t3i = ar - cr, ai - ci, br - dr, bi - di
    p, m = (t1r + t3i, t1i - t3r), (t1r - t3i, t1i + t3r)
    return [p, m] if sign < 0 else [m, p]


def _dft4(x, sign):
    y0, y2 = _dft4_half(x, sign, 0)
    y1, y3 = _dft4_half(x, sign, 1)
    return [y0, y1, y2, y3]


def _twid16(v, e, sign):
    r, i = v
    e = e % 16
    if e == 0:
        return v
    h = math.sqrt(0.5)
    if e == 4:
        return (-i, r) if sign > 0 else (i, -r)
    if e == 2:
        return (h * (r - i), h * (r + i)) if sign > 0 else (h * (r + i), h * (i - r))
    if e == 6:
        return (-h * (r + i), h * (r - i)) if sign > 0 else (h * (i - r), -h * (r + i))
    c = math.cos(2 * math.pi * e / 16)
    s = sign * math.sin(2 * math.pi * e / 16)
    return (c * r - s * i, s * r + c * i)


def _iota(shape, dim):
    return jax.lax.broadcasted_iota(jnp.int32, shape, dim)


def _cos_quarter(t):
    q = jnp.floor(t + 0.5)
    x = (t - q) * (math.pi / 2)
    x2 = x * x
    c = 1.0 + x2 * (-1.0 / 2 + x2 * (1.0 / 24 + x2 * (-1.0 / 720 + x2 * (1.0 / 40320))))
    s = x * (1.0 + x2 * (-1.0 / 6 + x2 * (1.0 / 120 + x2 * (-1.0 / 5040 + x2 * (1.0 / 362880)))))
    qi = q.astype(jnp.int32)
    v = jnp.where((qi & 1) == 1, s, c)
    return jnp.where(((qi + 1) & 2) == 2, -v, v)


def _expi_quarter(t):
    q = jnp.floor(t + 0.5)
    x = (t - q) * (math.pi / 2)
    x2 = x * x
    c = 1.0 + x2 * (-1.0 / 2 + x2 * (1.0 / 24 + x2 * (-1.0 / 720 + x2 * (1.0 / 40320))))
    s = x * (1.0 + x2 * (-1.0 / 6 + x2 * (1.0 / 120 + x2 * (-1.0 / 5040 + x2 * (1.0 / 362880)))))
    qi = q.astype(jnp.int32)
    odd = (qi & 1) == 1
    u = jnp.where(odd, s, c)
    v = jnp.where(odd, c, s)
    return jnp.where(((qi + 1) & 2) == 2, -u, u), jnp.where((qi & 2) == 2, v, -v)


def _dot(a, b):
    return jnp.dot(a, b, preferred_element_type=F32)


def _tile(n):
    return slice(128 * n, 128 * n + 128)


def _weave(*streams):
    live = [[g, n, 0] for g, n in streams if g is not None]
    while live:
        cur = min(live, key=lambda e: (e[2] + 0.5) / e[1])
        try:
            next(cur[0])
            cur[2] += 1
        except StopIteration:
            live.remove(cur)


def _scratch():
    v = lambda shape, dt: pltpu.VMEM((1,) + shape, dt)
    return dict(
        xio=pltpu.VMEM((S, D), BF16),
        wraw=pltpu.VMEM((640, S), BF16),
        wlast=pltpu.VMEM((4, 1, S), BF16),
        w1t=pltpu.VMEM((F, S), BF16),
        w2=pltpu.VMEM((F, S), BF16),
        b1v=pltpu.VMEM((F,), BF16),
        b2v=pltpu.VMEM((S,), BF16),
        wt1=[v((S // 2, 128), U32) for _ in range(5)],
        wt2=[v((4, 640, 128), U32) for _ in range(2)],
        eye=v((128, 128), BF16),
        wex=v((16, 2, 8, 128), F32),
        b1c=v((NFT * 128, 128), F32),
        ACC=[v((W1C, 128), F32) for _ in range(5)],
        XA=[v((D, 128), F32) for _ in range(NTT)],
        XB=[v((D, 128), F32) for _ in range(NTT)],
        YB=[v((5, 128, 128), BF16) for _ in range(NTT)],
        U=[v((2, r, S), F32) for r in _ROWS],
        XS=[v((2, r, S), F32) for r in _ROWS],
        V=[v((2, r, S), F32) for r in _ROWS],
        Q=[[v((4, 128, 128), F32) for _ in range(4)] for _ in range(5)],
        HB=[v((D, 128), BF16) for _ in range(NTT)],
        GB=[v((D // 2, 128), U32) for _ in range(NFT)],
        gf=v((16, 3, 128, 128), BF16),
        mf=v((5, 144, 128), BF16),
        mi=v((5, 128, 128), BF16),
        sem_x=pltpu.SemaphoreType.DMA((NTT,)),
        sem_w=pltpu.SemaphoreType.DMA((12,)),
        sem_w1=pltpu.SemaphoreType.DMA((NW1,)),
        sem_w2=pltpu.SemaphoreType.DMA((NW2,)),
        sem_o=pltpu.SemaphoreType.DMA((NTT + 2,)),
        sem_z=pltpu.SemaphoreType.REGULAR,
        sem_f=pltpu.SemaphoreType.REGULAR,
    )


def _is_leaf(x):
    return not isinstance(x, (dict, list))


def _kernel(x_hbm, wr_hbm, wi_hbm, w1t_hbm, b1_hbm, w2_hbm, b2_hbm, o_hbm, *scratch):
    sc = jax.tree_util.tree_unflatten(jax.tree_util.tree_structure(_scratch(), is_leaf=_is_leaf), scratch)
    xio, wraw, wlast, w1t, w2, b1_ref, b2_ref = (sc[k] for k in ("xio", "wraw", "wlast", "w1t", "w2", "b1v", "b2v"))
    wt1, wt2, wex, b1c, ACC = (sc[k] for k in ("wt1", "wt2", "wex", "b1c", "ACC"))
    XA, XB, YB, U, XS, V, Q, HB, GB = (sc[k] for k in ("XA", "XB", "YB", "U", "XS", "V", "Q", "HB", "GB"))
    gf, mf, mi = (sc[k] for k in ("gf", "mf", "mi"))
    sem_x, sem_w, sem_w1, sem_w2, sem_o = (sc[k] for k in ("sem_x", "sem_w", "sem_w1", "sem_w2", "sem_o"))

    def x_copy(t):
        return pltpu.make_async_copy(x_hbm.at[0, pl.ds(t * 128, 128), :], xio.at[pl.ds(t * 128, 128), :], sem_x.at[t])

    def o_copy(t, d0=0, d1=D, k=None):
        return pltpu.make_async_copy(xio.at[pl.ds(t * 128, 128), pl.ds(d0, d1 - d0)],
                                     o_hbm.at[0, pl.ds(t * 128, 128), pl.ds(d0, d1 - d0)],
                                     sem_o.at[t if k is None else k])

    w_parts = [[(wr_hbm, 0, 0, 128)], [(wr_hbm, 128, 128, 128)], [(wr_hbm, 256, 256, 64), (wi_hbm, 0, 320, 64)],
               [(wi_hbm, 64, 384, 128)], [(wi_hbm, 192, 512, 128)]]
    w_copies, n = [], 0
    for blk in w_parts:
        cur = []
        for (src, s0, d0, rows) in blk:
            cur.append(pltpu.make_async_copy(src.at[pl.ds(s0, rows), :], wraw.at[pl.ds(d0, rows), :], sem_w.at[n]))
            n += 1
        w_copies.append(cur)
    small = []
    for a, src in enumerate((wr_hbm, wi_hbm)):
        small.append(pltpu.make_async_copy(src.at[pl.ds(320, 1), :], wlast.at[a], sem_w.at[n]))
        n += 1
    for src, dst in ((b1_hbm, b1_ref), (b2_hbm, b2_ref)):
        small.append(pltpu.make_async_copy(src, dst, sem_w.at[n]))
        n += 1

    def w1_copy(i):
        rows = min(W1C, F - i * W1C)
        return pltpu.make_async_copy(w1t_hbm.at[pl.ds(i * W1C, rows), :], w1t.at[pl.ds(i * W1C, rows), :], sem_w1.at[i])

    def w2_copy(i):
        return pltpu.make_async_copy(w2_hbm.at[pl.ds(i * W2C, W2C), :], w2.at[pl.ds(i * W2C, W2C), :], sem_w2.at[i])

    seps = [pltpu.make_async_copy(wr_hbm.at[pl.ds(320, 1), :], wlast.at[2 + a], sem_w.at[n + a]) for a in range(2)]
    PR = 2
    cnt = [0]

    def go(cp, kind):
        if PR == 1:
            p = cnt[0] % 2 if kind == 'c' else 0
        elif PR == 2:
            p = 0 if kind == 'c' else 1
        elif PR == 3:
            p = 1 if kind == 'c' else 0
        else:
            p = 0
        cnt[0] += 1
        cp.start(priority=p)

    for seg in _XSEG:
        for t in seg:
            go(x_copy(t), 'c')
    for cp in small:
        go(cp, 'c')
    for blk in w_copies:
        for cp in blk:
            go(cp, 'c')
    go(seps[0], 'c')
    for i in range(NW1):
        go(w1_copy(i), 'b')
    go(seps[1], 'b')
    for i in range(NW2):
        go(w2_copy(i), 'b')

    zpool = [pl.semaphore_read(sc["sem_z"]) for _ in range(NZ)]
    lay = [0]

    def zz(i=0):
        return zpool[8 * lay[0] + i]

    def ldb(ref, z, *idx):
        return pltpu.bitcast(ref.bitcast(U32)[(z,) + idx], BF16)

    def fence():
        pl.semaphore_signal(sc["sem_f"], 1)
        pl.semaphore_wait(sc["sem_f"], 1)

    def d_tables():
        row = _iota((128, 128), 0)
        col = _iota((128, 128), 1)
        sc["eye"][0] = jnp.where(row == col, 1.0, 0.0).astype(BF16)
        n2 = col & 63
        is_b = col >= 64
        is_im = (row & 8) == 8
        rr = ((row >> 4) << 3) | (row & 7)
        j = rr & 31
        second = rr >= 32
        for g in range(5):
            ra, rb = _RES[g]
            kb = jnp.where(second, rb, ra) + 10 * j
            idx = kb * n2
            if g == 0:
                idx = idx + jnp.where(is_im, 160, 0)
                amp = jnp.where(second == is_b, 1.0, 0.0).astype(F32)
            else:
                idx = idx + jnp.where(is_im != is_b, 160, 0)
                sg = jnp.where((rb == _BASE[g]) == second, 1.0, -1.0).astype(F32)
                amp = jnp.where(is_b, jnp.where(is_im, -sg * _SC[g], sg * _SC[g]), 1.0).astype(F32)
            m = amp * _cos_quarter(idx.astype(F32) * (1.0 / 160))
            mf[0, g, 0:128, :] = m.astype(BF16)
            mt = m * (2.0 / (S * D))
            if g == 0:
                mt = jnp.where(kb == 0, 0.5 * mt, mt)
                nyq = jnp.where(is_b, 0.0, jnp.where((n2 & 1) == 0, 1.0, -1.0)).astype(F32)
                mt = jnp.where(row == 8, nyq * (1.0 / (S * D)), mt)
                r16 = _iota((16, 128), 0)
                c16 = _iota((16, 128), 1)
                ext = jnp.where((r16 == 0) & (c16 < 64), jnp.where((c16 & 1) == 0, 1.0, -1.0), 0.0).astype(F32)
                mf[0, 0, 128:144, :] = ext.astype(BF16)
            mi[0, g] = mt.T.astype(BF16)

    def s_tables():
        col = _iota((16, 128), 1)
        k2 = 8 * (col & 15) + (col >> 4)

        def strip(i, carry):
            row = _iota((16, 128), 0) + 16 * i
            ga, gb = _expi_quarter(((row * k2) & 127).astype(F32) * (1.0 / 32))
            ta, tb = _expi_quarter(row.astype(F32) * (1.0 / 512))
            rs = pl.ds(pl.multiple_of(16 * i, 16), 16)
            for k1 in range(16):
                gf[0, k1, 0, rs, :] = ga.astype(BF16)
                gf[0, k1, 1, rs, :] = (gb - ga).astype(BF16)
                gf[0, k1, 2, rs, :] = (ga + gb).astype(BF16)
                if k1 < 15:
                    ga, gb = ga * ta - gb * tb, ga * tb + gb * ta
            return carry

        jax.lax.fori_loop(0, 8, strip, 0, unroll=2)

    def w_t1(b):
        for jt in range(16):
            blk = pltpu.bitcast(wraw[_tile(b), _tile(jt)].T, U32)
            for a in range(8):
                pos = 8 * (16 * a + jt)
                wt1[b][0, pos: pos + 8, :] = blk[8 * a: 8 * a + 8]
            yield

    def w_t2(b):
        z = zz()
        for m in (0, 2, 4, 6, 1, 3, 5, 7):
            wt2[m % 2][0, m // 2, _tile(b), :] = wt1[b][z, pl.ds(m, 128, stride=8), :].T
            yield

    def w_extra():
        r8 = _iota((8, S), 0)
        lane = _iota((8, 128), 1)
        e = jnp.where(r8 == 0, jnp.broadcast_to(wlast[0].astype(F32), (8, S)),
                      jnp.where(r8 == 1, jnp.broadcast_to(wlast[1].astype(F32), (8, S)), 0.0))
        v = [e[:, _tile(n)] for n in range(16)]
        for b in range(4):
            stp = 1 << b
            msk = (lane & stp) == 0
            for n in range(16):
                if n & stp:
                    continue
                lo, hi = v[n], v[n | stp]
                v[n] = jnp.where(msk, lo, pltpu.roll(hi, stp, 1))
                v[n | stp] = jnp.where(msk, pltpu.roll(lo, 128 - stp, 1), hi)
            yield
        r = _iota((8, 128), 0)
        for n in range(16):
            wex[0, n, 0] = jnp.where(r == 0, v[n], 0.0)
            wex[0, n, 1] = jnp.where(r == 0, pltpu.roll(v[n], 7, 0), 0.0)
        yield

    bias = {}

    def bias_prep():
        bias[2] = b2_ref[...].astype(F32).reshape(1, S)
        b1 = b1_ref[...].astype(F32).reshape(1, F)
        b1 = jnp.concatenate([b1, jnp.zeros((1, NFT * 128 - F), F32)], axis=1)
        for j in range(NFT):
            b1c[0, _tile(j), :] = jnp.broadcast_to(b1[:, _tile(j)], (128, 128)).T
            yield

    rstd, mean, x_done, outs = {}, {}, set(), []

    def ld(src, z, rs, n):
        return (src[z, 0, rs, _tile(n)], src[z, 1, rs, _tile(n)])

    def st(dst, rs, n, v):
        dst[0, 0, rs, _tile(n)] = v[0]
        dst[0, 1, rs, _tile(n)] = v[1]

    def x_in(tiles):
        for t in tiles:
            for j in range(5):
                if XMXU:
                    XA[t][0, _tile(j), :] = jax.lax.dot_general(
                        ldb(sc["eye"], zz(t % 8)), xio[_tile(t), _tile(j)], NT, preferred_element_type=F32)
                else:
                    XA[t][0, _tile(j), :] = xio[_tile(t), _tile(j)].T.astype(F32)
                if j == 4:
                    x_done.add(t)
                yield

    def front_vpu(tiles):
        for t in tiles:
            z = zz()
            e0s, ssq = [], None
            for rp in range(4):
                xs = [XA[t][z, 64 * n + 16 * rp: 64 * n + 16 * rp + 16, :] for n in range(10)]
                sm = [xs[n] + xs[n + 5] for n in range(5)]
                df = [xs[n] - xs[n + 5] if n % 2 == 0 else xs[n + 5] - xs[n] for n in range(5)]
                e0, e1r, e1i, e2r, e2i = _dft5(sm)
                o0, o1r, o1i, o2r, o2i = _dft5(df)
                q = (0.5 * (o0 * o0) + (e1r * e1r + e2r * e2r + o1r * o1r + o2r * o2r)
                     + (_S1 * _S1) * (e1i * e1i + o1i * o1i) + (_S2 * _S2) * (e2i * e2i + o2i * o2i))
                ssq = q if ssq is None else ssq + q
                e0s.append(e0)
                a, b = slice(16 * rp, 16 * rp + 16), slice(64 + 16 * rp, 64 + 16 * rp + 16)
                YB[t][0, 0, b, :] = o0.astype(BF16)
                for g, (va, vb) in enumerate(((o2r, o2i), (e1r, e1i), (o1r, o1i), (e2r, e2i))):
                    YB[t][0, g + 1, a, :] = va.astype(BF16)
                    YB[t][0, g + 1, b, :] = vb.astype(BF16)
                if rp < 3:
                    yield
            tot = jnp.sum(e0s[0] + e0s[1] + e0s[2] + e0s[3], axis=0, keepdims=True)
            mu10 = tot * (1.0 / 64)
            mean[t] = tot * (1.0 / D)
            e0s = [e - mu10 for e in e0s]
            q0 = e0s[0] * e0s[0] + e0s[1] * e0s[1] + e0s[2] * e0s[2] + e0s[3] * e0s[3]
            var = jnp.sum(ssq + 0.5 * q0, axis=0, keepdims=True) * (2.0 / (10 * D))
            rstd[t] = jax.lax.rsqrt(var + EPS)
            for rp in range(4):
                YB[t][0, 0, 16 * rp: 16 * rp + 16, :] = e0s[rp].astype(BF16)
            yield

    def front_mxu(b):
        z = zz(b)
        for g in range(5):
            lhs = ldb(mf, z, 0) if g == 0 else ldb(mf, z, g, slice(0, 64))
            y = _dot(lhs, jnp.concatenate([ldb(YB[4 * a + b], z, g) for a in range(4)], axis=1))
            sc_ = lambda r0, a: y[r0: r0 + 8, _tile(a)] * rstd[4 * a + b]
            for i in range(9 if g == 0 else 8):
                if i < 8:
                    xs = [(sc_(16 * i, a), sc_(16 * i + 8, a)) for a in range(4)]
                else:
                    xs = [(sc_(128, a), jnp.zeros((8, 128), F32)) for a in range(4)]
                t = _dft4(xs, -1)
                for ka in range(4):
                    st(U[g], slice(8 * i, 8 * i + 8), 4 * ka + b, _twid16(t[ka], b * ka, -1))
            yield

    def pass_f(gs):
        zt = zz(gs[0])
        cat = lambda vs: jnp.concatenate(vs, axis=0) if len(vs) > 1 else vs[0]
        for ka in range(4):
            for par in range(2):
                xs = []
                for b in range(4):
                    pr = [ld(U[g], zz(par), slice(0, _ROWS[g]), 4 * ka + b) for g in gs]
                    xs.append((cat([p[0] for p in pr]), cat([p[1] for p in pr])))
                for h, (ur, ui) in enumerate(_dft4_half(xs, -1, par)):
                    k1 = ka + 4 * (par + 2 * h)
                    p1 = _dot((ur + ui).astype(BF16), ldb(gf, zt, k1, 0))
                    p2 = _dot(ur.astype(BF16), ldb(gf, zt, k1, 1))
                    p3 = _dot(ui.astype(BF16), ldb(gf, zt, k1, 2))
                    xr, xi = p1 - p3, p1 + p2
                    r0 = 0
                    for g in gs:
                        st(XS[g], slice(0, _ROWS[g]), k1, (xr[r0: r0 + _ROWS[g]], xi[r0: r0 + _ROWS[g]]))
                        r0 += _ROWS[g]
                yield

    def w_rows(z, a, g, k1):
        parts = []
        for res in _RES[g]:
            blk = wt2[(k1 // 2) % 2][z, k1 // 4, pl.ds(320 * a + res, 32, stride=10), :]
            blk = (blk << 16) if k1 % 2 == 0 else (blk & jnp.uint32(0xFFFF0000))
            parts.append(pltpu.bitcast(blk, F32))
        if g == 0:
            parts.append(jnp.concatenate([wex[z, k1, a], jnp.zeros((8, 128), F32)], axis=0))
        return parts

    def pass_i(g):
        if MIR == 64:
            blocks = [(0, _ROWS[g], (0, 1, 2) if g == 0 else (0, 1))]
        else:
            blocks = [(0, 32, (0,)), (32, _ROWS[g], (1, 2) if g == 0 else (1,))]
        for ka in range(4):
            for bi, (r0, r1, wsel) in enumerate(blocks):
                z = zz((g + 3 + 5 * bi) % 8)
                rs = slice(r0, r1)
                vs = []
                for kb in range(4):
                    k1 = ka + 4 * kb
                    xr, xi = ld(XS[g], z, rs, k1)
                    wr, wi = [jnp.concatenate([p for q, p in enumerate(w_rows(z, a, g, k1)) if q in wsel], axis=0)
                              for a in range(2)]
                    yr = xr * wr - xi * wi
                    yi = xr * wi + xi * wr
                    dt = lambda a, j: jax.lax.dot_general(a.astype(BF16), ldb(gf, z, k1, j), NT,
                                                          preferred_element_type=F32)
                    q1 = dt(yr + yi, 0)
                    q2 = dt(yi, 1)
                    q3 = dt(yr, 2)
                    vs.append((q1 + q2, q1 - q3))
                    if kb == 1 and len(blocks) == 1:
                        yield
                t = _dft4(vs, +1)
                for b in range(4):
                    st(V[g], rs, 4 * ka + b, _twid16(t[b], b * ka, +1))
                yield

    def pass_b(g, bs=range(4)):
        for b in bs:
            z = zz(b)
            rhs = [[] for _ in range(4)]
            for i in range(8):
                rs = slice(8 * i, 8 * i + 8)
                y = _dft4([ld(V[g], z, rs, 4 * ka + b) for ka in range(4)], +1)
                if g == 0 and i == 0:
                    r8 = _iota((8, 128), 0)
                    ex = _dft4([ld(V[0], z, slice(64, 72), 4 * ka + b) for ka in range(4)], +1)
                    y = [(y[a][0], jnp.where(r8 == 0, ex[a][0], y[a][1])) for a in range(4)]
                for a in range(4):
                    rhs[a] += [y[a][0], y[a][1]]
            yield
            for a in range(4):
                Q[g][b][0, a] = _dot(ldb(mi, z, g), jnp.concatenate(rhs[a], axis=0).astype(BF16))
            yield

    def back_vpu(tiles):
        for t in tiles:
            z = zz(1)
            qa, qb = t // 4, t % 4
            q = lambda g, rs: Q[g][qb][z, qa, rs, :]
            q0 = [q(0, slice(8 * rp, 8 * rp + 8)) for rp in range(8)]
            qs = ((q0[0] + q0[1]) + (q0[2] + q0[3])) + ((q0[4] + q0[5]) + (q0[6] + q0[7]))
            mu = mean[t] + jnp.sum(qs, axis=0, keepdims=True) * (10.0 / D)
            mean[t] = mu
            s2 = [None, None]
            for rp in range(8):
                a, b = slice(8 * rp, 8 * rp + 8), slice(64 + 8 * rp, 64 + 8 * rp + 8)
                e = _dft5_t(q0[rp] - mu, q(2, a), q(2, b), q(4, a), q(4, b))
                o = _dft5_t(q(0, b), q(3, a), q(3, b), q(1, a), q(1, b))
                for n in range(5):
                    lo = slice(64 * n + 8 * rp, 64 * n + 8 * rp + 8)
                    hi = slice(64 * (n + 5) + 8 * rp, 64 * (n + 5) + 8 * rp + 8)
                    if n % 2 == 0:
                        ylo, yhi = e[n] + o[n], e[n] - o[n]
                    else:
                        ylo, yhi = e[n] - o[n], e[n] + o[n]
                    xlo = XA[t][z, lo, :] + ylo
                    xhi = XA[t][z, hi, :] + yhi
                    XB[t][0, lo, :] = xlo
                    XB[t][0, hi, :] = xhi
                    s2[0] = xlo * xlo if s2[0] is None else s2[0] + xlo * xlo
                    s2[1] = xhi * xhi if s2[1] is None else s2[1] + xhi * xhi
                if rp % 2 == 1:
                    yield
            var = jnp.sum(s2[0] + s2[1], axis=0, keepdims=True) * (1.0 / D)
            r1 = jax.lax.rsqrt(var + EPS)
            r2 = jax.lax.rsqrt(var * r1 * r1 + EPS)
            rr = r1 * r2
            for i in range(D // 16):
                HB[t][0, 16 * i: 16 * i + 16, :] = (XB[t][z, 16 * i: 16 * i + 16, :] * rr).astype(BF16)
            yield

    def act(get, off, w, zi):
        z = zz(zi)
        for r0 in range(0, w, 128):
            r1 = min(r0 + 128, w)
            j = (off + r0) // 128
            for i in range(5):
                parts = []
                for q in range(r0, r1, 32):
                    u = get(q, q + 32, i) + b1c[z, off + q: off + q + 32, :]
                    parts.append(jax.nn.gelu(u, approximate=True))
                g = jnp.concatenate(parts, axis=0).astype(BF16).T
                GB[j][0, 64 * i: 64 * i + 64, 0: r1 - r0] = pltpu.bitcast(g, U32)
                yield

    def mm1_dot(off, w, zi):
        z = zz(zi)
        rhs = jnp.concatenate([ldb(HB[t], z) for t in range(NTT)], axis=1)
        u = jax.lax.dot_general(w1t[off: off + w, :], rhs, NT, preferred_element_type=F32)
        return lambda r0, r1, i: u[r0:r1, _tile(i)]

    def mm1_step(tiles, first):
        z = zz()
        lhs = jnp.concatenate([w1t[0:W1C, _tile(t)] for t in tiles], axis=1)
        for i in range(5):
            rhs = jnp.concatenate([ldb(HB[t], z, slice(64 * i, 64 * i + 64)) for t in tiles], axis=1)
            part = jax.lax.dot_general(lhs, rhs, NT, preferred_element_type=F32)
            ACC[i][0] = part if first else ACC[i][z] + part
            yield

    def mm2(c, tiles, d0=0, d1=D):
        z = zz(c % 8)
        rs = slice(d0 // 2, d1 // 2)
        parts = [GB[j][z, rs, :] for j in range(NFT - 1)] + [GB[NFT - 1][z, rs, 0: F % 128]]
        y = _dot(jnp.concatenate([pltpu.bitcast(p, BF16) for p in parts], axis=1),
                 jnp.concatenate([w2[:, _tile(t)] for t in tiles], axis=1))
        return [XB[t][zz(2), d0:d1, :] + (y[:, _tile(i)] + (bias[2][:, _tile(t)] + mean[t]))
                for i, t in enumerate(tiles)]

    def scope(name):
        return contextlib.nullcontext()

    with scope("p0_tables"):
        d_tables()
        U[0][0, :, 72:80, :] = jnp.zeros((2, 8, S), F32)
        s_tables()
    with scope("p1_front"):
        nseg = len(_XSEG)
        pend_v, fv_done, fm_done = [], [], []
        for c in range(nseg):
            with scope("wx%d" % c):
                for t in _XSEG[c]:
                    x_copy(t).wait()
            if c == nseg - 1:
                with scope("ww0"):
                    for cp in small:
                        cp.wait()
            last = c == nseg - 1
            ready = [b for b in range(3) if b not in fm_done and all(4 * a + b in fv_done for a in range(4))]
            fm_done += ready
            cand = pend_v + _XSEG[c]
            keep = 0 if last else min(LAG, len(cand))
            fv, pend_v = cand[:len(cand) - keep], cand[len(cand) - keep:]
            fv_done += fv
            extra = []
            if c == nseg - 1:
                extra = [(w_extra(), 5)]
            xg = x_in(_XSEG[c])

            def fv_gen(tiles, xg=xg):
                for t in tiles:
                    while t not in x_done:
                        next(xg)
                    yield from front_vpu([t])

            _weave((xg, 5 * len(_XSEG[c])),
                   (fv_gen(fv) if fv else None, 4 * max(len(fv), 1) + 2),
                   (itertools.chain(*[front_mxu(b) for b in ready]) if ready else None, 5), *extra)
        _weave((itertools.chain(*[front_mxu(b) for b in range(4) if b not in fm_done]), 5))
    for layer in range(2):
        lay[0] = layer
        with scope("p2_F%d" % layer):
            if layer == 0:
                plan = (((0, 1), (0, 1), [w_t1(0), w_t1(1), w_t2(0), w_t2(1)], 48),
                        ((2, 3), (2, 3), [w_t1(2), w_t1(3), w_t2(2), w_t2(3)], 48),
                        ((4,), (4,), [w_t1(4), w_t2(4)], 24))
                for gs, ws, xl, nx in plan:
                    with scope("ww%d" % ws[-1]):
                        for r in ws:
                            for cp in w_copies[r]:
                                cp.wait()
                    _weave((pass_f(gs), 8), (itertools.chain(*xl), nx))
            else:
                if 'a' in FENCES:
                    fence()
                for gs in ((0, 1), (2, 3, 4)):
                    _weave((pass_f(gs), 8))
                if 'b' in FENCES:
                    fence()
        with scope("p3_I%d" % layer):
            for r in range(5):
                _weave((pass_i(r), 8), (pass_b(r - 1) if 1 <= r < 4 else None, 8))
            if layer == 0:
                w1_copy(0).wait()
            elif 'c' in FENCES:
                fence()
        with scope("p4_back%d" % layer):
            _weave((pass_b(4, [0]), 2), (pass_b(3, [0]), 2))
            rest = itertools.chain(*[pass_b(g, [b]) for b in (1, 2, 3) for g in (3, 4)])
            P = _PAIRS
            steps = {1: P[0], 2: P[1], 4: P[2] + P[3], 6: P[4] + P[5], 8: P[6] + P[7]} if STEP4 else \
                {i: P[i - 1] for i in range(1, 9)}
            i = 0
            while i <= len(P):
                span = 2 if (STEP4 and i in (2, 4, 6)) else 1
                tiles = [t for q in range(i, min(i + span, len(P))) for t in P[q]]
                _weave((rest if i == 0 else None, 12),
                       (back_vpu(tiles) if tiles else None, 5 * max(len(tiles), 1)),
                       (mm1_step(steps[i], i == 1) if i in steps else None, 5),
                       (bias_prep() if layer == 0 and i == len(P) else None, NFT))
                i += span
            if layer == 0:
                for i in range(1, NW1):
                    w1_copy(i).wait()
                if STOP == 'A1':
                    xio[0:W1C, 0:640] = jnp.concatenate([ACC[i][zz(3)] for i in range(5)], axis=1).astype(BF16)
                    for t in range(3):
                        o_copy(t).start()
                    for t in range(3):
                        o_copy(t).wait()
                    for i in range(NW2):
                        w2_copy(i).wait()
                    for cp in seps:
                        cp.wait()
                    return
            elif 'd' in FENCES:
                fence()
        with scope("p5_mm_%d" % layer):
            za = zz(1)
            pend = (lambda r0, r1, i: ACC[i][za, r0:r1, :], 0, W1C, 0)
            off = W1C
            for i, w in enumerate(W1S):
                if layer == 0 and i == len(W1S) - 1:
                    for ii in range(NW2):
                        w2_copy(ii).wait()
                    for cp in seps:
                        cp.wait()
                cur = (mm1_dot(off, w, i + 1), off, w, i + 1)
                _weave((act(*pend), 1))
                pend = cur
                off += w
            assert off == F
            _weave((act(*pend), 1))
            nch = len(_PAIRS)
            if STOP.startswith('B'):
                for c in range(int(STOP[1:])):
                    for t, v in zip(_PAIRS[c], mm2(c, _PAIRS[c])):
                        xio[_tile(t), :] = v.astype(BF16).T
                for t in range(NTT):
                    o_copy(t).start()
                for t in range(NTT):
                    o_copy(t).wait()
                return
            if layer == 0:
                for c in range(nch + 1):
                    if c < nch:
                        for t, v in zip(_PAIRS[c], mm2(c, _PAIRS[c])):
                            XA[t][0] = v
                    lay[0] = 1
                    if c == nch:
                        _weave((front_mxu(2), 5), (front_vpu(_PAIRS[c - 1]), 8))
                    elif c >= 1:
                        _weave((front_vpu(_PAIRS[c - 1]), 8))
                    if c in (2, 4, nch):
                        _weave((front_mxu(c // 2 - 1), 5))
                    lay[0] = 0
            else:
                jobs = [(c, _PAIRS[c], 0, D) for c in range(nch - 1)]
                jobs += [(nch - 1, _PAIRS[-1], 0, DS), (nch, _PAIRS[-1], DS, D)]
                prev = None
                for n, job in enumerate(jobs + [None]):
                    cur = (job, mm2(*job)) if job is not None else None
                    if prev is not None:
                        (_, tiles, d0, d1), vals = prev
                        for i, (t, v) in enumerate(zip(tiles, vals)):
                            xio[_tile(t), d0:d1] = v.astype(BF16).T
                            outs.append(o_copy(t, d0, d1, NTT + i if d0 else None))
                            outs[-1].start()
                        if n in (nch - 2, nch):
                            fence()
                    prev = cur

    with scope("p7_out"):
        for cp in outs:
            cp.wait()


@jax.jit
def pallas_interleave_layers__spectral_gfnet__mixer_token_mlp__prompt_kernel(A_x, A_w_r, A_w_i, B_x, B_w1, B_b1, B_w2, B_b2):
    del B_x
    any_spec = pl.BlockSpec(memory_space=pl.ANY)
    return pl.pallas_call(
        _kernel,
        out_shape=jax.ShapeDtypeStruct((1, S, D), BF16),
        in_specs=[any_spec] * 7,
        out_specs=any_spec,
        scratch_shapes=jax.tree_util.tree_leaves(_scratch(), is_leaf=_is_leaf),
        compiler_params=pltpu.CompilerParams(vmem_limit_bytes=120 * 1024 * 1024),
    )(A_x, A_w_r.T, A_w_i.T, B_w1.T, B_b1, B_w2, B_b2)
```

```python
import itertools
import math

import jax
import jax.numpy as jnp
import jax.experimental.pallas as pl
import jax.experimental.pallas.tpu as pltpu

S = 2048
D = 640
F = 1728
EPS = 1e-5
F32 = jnp.float32
BF16 = jnp.bfloat16
U32 = jnp.uint32
NT = (((1,), (1,)), ((), ()))

_C1, _C2 = math.cos(2 * math.pi / 5), math.cos(4 * math.pi / 5)
_S1, _S2 = math.sin(2 * math.pi / 5), math.sin(4 * math.pi / 5)
_KN = (_C1 - _C2) / 2
_RES = ((0, 5), (1, 9), (2, 8), (3, 7), (4, 6))
_BASE = (None, 9, 2, 7, 4)
_SC = (None, _S2, _S1, _S1, _S2)
_ROWS = (80, 64, 64, 64, 64)

W1C = 640
W1S = (384, 384, 320)
NW1 = -(-F // W1C)
W2C = 216
NW2 = F // W2C
NFT = -(-F // 128)
NTT = S // 128
NZ = 16
DS = 512
_PAIRS = [(b + 8 * h, b + 8 * h + 4) for b in range(4) for h in range(2)]
_XSEG = [[0, 4, 8, 12], [1, 5, 9, 13], [2, 6], [10, 14], [3, 7], [11, 15]]


def _dft5(a):
    a1 = a[1] + a[4]
    b1 = a[1] - a[4]
    a2 = a[2] + a[3]
    b2 = a[2] - a[3]
    t = a1 + a2
    y0 = a[0] + t
    m = a[0] - 0.25 * t
    n = _KN * (a1 - a2)
    return y0, m + n, b1 + (_S2 / _S1) * b2, m - n, b1 - (_S1 / _S2) * b2


def _dft5_t(y0, y1r, y1i, y2r, y2i):
    gm = y1r + y2r
    gn = _KN * (y1r - y2r)
    a0 = y0 + gm
    gt = y0 - 0.25 * gm
    ga1 = gt + gn
    ga2 = gt - gn
    gb1 = y1i + y2i
    gb2 = (_S2 / _S1) * y1i - (_S1 / _S2) * y2i
    return [a0, ga1 + gb1, ga2 + gb2, ga2 - gb2, ga1 - gb1]


def _dft4_half(x, sign, par):
    (ar, ai), (br, bi), (cr, ci), (dr, di) = x
    if par == 0:
        t0r, t0i, t2r, t2i = ar + cr, ai + ci, br + dr, bi + di
        return [(t0r + t2r, t0i + t2i), (t0r - t2r, t0i - t2i)]
    t1r, t1i, t3r, t3i = ar - cr, ai - ci, br - dr, bi - di
    p, m = (t1r + t3i, t1i - t3r), (t1r - t3i, t1i + t3r)
    return [p, m] if sign < 0 else [m, p]


def _dft4(x, sign):
    y0, y2 = _dft4_half(x, sign, 0)
    y1, y3 = _dft4_half(x, sign, 1)
    return [y0, y1, y2, y3]


def _twid16(v, e, sign):
    r, i = v
    e = e % 16
    if e == 0:
        return v
    h = math.sqrt(0.5)
    if e == 4:
        return (-i, r) if sign > 0 else (i, -r)
    if e == 2:
        return (h * (r - i), h * (r + i)) if sign > 0 else (h * (r + i), h * (i - r))
    if e == 6:
        return (-h * (r + i), h * (r - i)) if sign > 0 else (h * (i - r), -h * (r + i))
    c = math.cos(2 * math.pi * e / 16)
    s = sign * math.sin(2 * math.pi * e / 16)
    return (c * r - s * i, s * r + c * i)


def _iota(shape, dim):
    return jax.lax.broadcasted_iota(jnp.int32, shape, dim)


def _cos_quarter(t):
    q = jnp.floor(t + 0.5)
    x = (t - q) * (math.pi / 2)
    x2 = x * x
    c = 1.0 + x2 * (-1.0 / 2 + x2 * (1.0 / 24 + x2 * (-1.0 / 720 + x2 * (1.0 / 40320))))
    s = x * (1.0 + x2 * (-1.0 / 6 + x2 * (1.0 / 120 + x2 * (-1.0 / 5040 + x2 * (1.0 / 362880)))))
    qi = q.astype(jnp.int32)
    v = jnp.where((qi & 1) == 1, s, c)
    return jnp.where(((qi + 1) & 2) == 2, -v, v)


def _expi_quarter(t):
    q = jnp.floor(t + 0.5)
    x = (t - q) * (math.pi / 2)
    x2 = x * x
    c = 1.0 + x2 * (-1.0 / 2 + x2 * (1.0 / 24 + x2 * (-1.0 / 720 + x2 * (1.0 / 40320))))
    s = x * (1.0 + x2 * (-1.0 / 6 + x2 * (1.0 / 120 + x2 * (-1.0 / 5040 + x2 * (1.0 / 362880)))))
    qi = q.astype(jnp.int32)
    odd = (qi & 1) == 1
    u = jnp.where(odd, s, c)
    v = jnp.where(odd, c, s)
    return jnp.where(((qi + 1) & 2) == 2, -u, u), jnp.where((qi & 2) == 2, v, -v)


def _gelu(x):
    c = math.sqrt(2 / math.pi)
    h = 0.5 * x
    return h + h * jnp.tanh(x * (c + (c * 0.044715) * (x * x)))


def _dot(a, b):
    return jnp.dot(a, b, preferred_element_type=F32)


def _tile(n):
    return slice(128 * n, 128 * n + 128)


def _weave(*streams):
    live = [[g, n, 0] for g, n in streams if g is not None]
    while live:
        cur = min(live, key=lambda e: (e[2] + 0.5) / e[1])
        try:
            next(cur[0])
            cur[2] += 1
        except StopIteration:
            live.remove(cur)


def _scratch():
    v = lambda shape, dt: pltpu.VMEM((1,) + shape, dt)
    return dict(
        xio=pltpu.VMEM((S, D), BF16),
        wraw=pltpu.VMEM((640, S), BF16),
        wlast=pltpu.VMEM((4, 1, S), BF16),
        w1t=pltpu.VMEM((F, S), BF16),
        w2=pltpu.VMEM((F, S), BF16),
        b1v=pltpu.VMEM((F,), BF16),
        b2v=pltpu.VMEM((S,), BF16),
        wt1=[v((S // 2, 128), U32) for _ in range(5)],
        wt2=[v((4, 640, 128), U32) for _ in range(2)],
        wex=v((16, 2, 8, 128), F32),
        b1c=v((NFT * 128, 128), F32),
        ACC=[v((W1C, 128), F32) for _ in range(5)],
        XA=[v((D, 128), F32) for _ in range(NTT)],
        XB=[v((D, 128), F32) for _ in range(NTT)],
        YB=[v((5, 128, 128), BF16) for _ in range(NTT)],
        U=[v((2, r, S), F32) for r in _ROWS],
        XS=[v((2, r, S), F32) for r in _ROWS],
        V=[v((2, r, S), F32) for r in _ROWS],
        Q=[[v((4, 128, 128), F32) for _ in range(4)] for _ in range(5)],
        HB=[v((D, 128), BF16) for _ in range(NTT)],
        GB=[v((D // 2, 128), U32) for _ in range(NFT)],
        gf=v((16, 3, 128, 128), BF16),
        mf=v((5, 144, 128), BF16),
        mi=v((5, 128, 128), BF16),
        sem_x=pltpu.SemaphoreType.DMA((NTT,)),
        sem_w=pltpu.SemaphoreType.DMA((12,)),
        sem_w1=pltpu.SemaphoreType.DMA((NW1,)),
        sem_w2=pltpu.SemaphoreType.DMA((NW2,)),
        sem_o=pltpu.SemaphoreType.DMA((NTT + 2,)),
        zv=pltpu.VMEM((8, 128), jnp.int32),
        zs=pltpu.SMEM((8, 128), jnp.int32),
        sem_z=pltpu.SemaphoreType.DMA,
        sem_f=pltpu.SemaphoreType.REGULAR,
    )


def _is_leaf(x):
    return not isinstance(x, (dict, list))


def _kernel(x_hbm, wr_hbm, wi_hbm, w1t_hbm, b1_hbm, w2_hbm, b2_hbm, o_hbm, *scratch):
    sc = jax.tree_util.tree_unflatten(jax.tree_util.tree_structure(_scratch(), is_leaf=_is_leaf), scratch)
    xio, wraw, wlast, w1t, w2, b1_ref, b2_ref = (sc[k] for k in ("xio", "wraw", "wlast", "w1t", "w2", "b1v", "b2v"))
    wt1, wt2, wex, b1c, ACC = (sc[k] for k in ("wt1", "wt2", "wex", "b1c", "ACC"))
    XA, XB, YB, U, XS, V, Q, HB, GB = (sc[k] for k in ("XA", "XB", "YB", "U", "XS", "V", "Q", "HB", "GB"))
    gf, mf, mi = (sc[k] for k in ("gf", "mf", "mi"))
    sem_x, sem_w, sem_w1, sem_w2, sem_o = (sc[k] for k in ("sem_x", "sem_w", "sem_w1", "sem_w2", "sem_o"))

    def x_copy(t):
        return pltpu.make_async_copy(x_hbm.at[0, pl.ds(t * 128, 128), :], xio.at[pl.ds(t * 128, 128), :], sem_x.at[t])

    def o_copy(t, d0=0, d1=D, k=None):
        return pltpu.make_async_copy(xio.at[pl.ds(t * 128, 128), pl.ds(d0, d1 - d0)],
                                     o_hbm.at[0, pl.ds(t * 128, 128), pl.ds(d0, d1 - d0)],
                                     sem_o.at[t if k is None else k])

    w_parts = [[(wr_hbm, 0, 0, 128)], [(wr_hbm, 128, 128, 128)], [(wr_hbm, 256, 256, 64), (wi_hbm, 0, 320, 64)],
               [(wi_hbm, 64, 384, 128)], [(wi_hbm, 192, 512, 128)]]
    w_copies, n = [], 0
    for blk in w_parts:
        cur = []
        for (src, s0, d0, rows) in blk:
            cur.append(pltpu.make_async_copy(src.at[pl.ds(s0, rows), :], wraw.at[pl.ds(d0, rows), :], sem_w.at[n]))
            n += 1
        w_copies.append(cur)
    small = []
    for a, src in enumerate((wr_hbm, wi_hbm)):
        small.append(pltpu.make_async_copy(src.at[pl.ds(320, 1), :], wlast.at[a], sem_w.at[n]))
        n += 1
    for src, dst in ((b1_hbm, b1_ref), (b2_hbm, b2_ref)):
        small.append(pltpu.make_async_copy(src, dst, sem_w.at[n]))
        n += 1

    def w1_copy(i):
        rows = min(W1C, F - i * W1C)
        return pltpu.make_async_copy(w1t_hbm.at[pl.ds(i * W1C, rows), :], w1t.at[pl.ds(i * W1C, rows), :], sem_w1.at[i])

    def w2_copy(i):
        return pltpu.make_async_copy(w2_hbm.at[pl.ds(i * W2C, W2C), :], w2.at[pl.ds(i * W2C, W2C), :], sem_w2.at[i])

    seps = [pltpu.make_async_copy(wr_hbm.at[pl.ds(320, 1), :], wlast.at[2 + a], sem_w.at[n + a]) for a in range(2)]

    sc["zv"][...] = jnp.zeros((8, 128), jnp.int32)
    z_copy = pltpu.make_async_copy(sc["zv"], sc["zs"], sc["sem_z"])
    z_copy.start()
    for cp in [x_copy(t) for seg in _XSEG for t in seg] + small + [cp for blk in w_copies for cp in blk] + seps[:1]:
        cp.start()
    for cp in [w1_copy(i) for i in range(NW1)] + seps[1:] + [w2_copy(i) for i in range(NW2)]:
        cp.start(priority=1)

    zpool = []
    lay = [0]

    def zz(i=0):
        return zpool[8 * lay[0] + i]

    def ldb(ref, z, *idx):
        return pltpu.bitcast(ref.bitcast(U32)[(z,) + idx], BF16)

    def fence():
        pl.semaphore_signal(sc["sem_f"], 1)
        pl.semaphore_wait(sc["sem_f"], 1)

    def d_tables():
        row = _iota((128, 128), 0)
        col = _iota((128, 128), 1)
        n2 = col & 63
        is_b = col >= 64
        is_im = (row & 8) == 8
        rr = ((row >> 4) << 3) | (row & 7)
        j = rr & 31
        second = rr >= 32
        for g in range(5):
            ra, rb = _RES[g]
            kb = jnp.where(second, rb, ra) + 10 * j
            idx = kb * n2
            if g == 0:
                idx = idx + jnp.where(is_im, 160, 0)
                amp = jnp.where(second == is_b, 1.0, 0.0).astype(F32)
            else:
                idx = idx + jnp.where(is_im != is_b, 160, 0)
                sg = jnp.where((rb == _BASE[g]) == second, 1.0, -1.0).astype(F32)
                amp = jnp.where(is_b, jnp.where(is_im, -sg * _SC[g], sg * _SC[g]), 1.0).astype(F32)
            m = amp * _cos_quarter(idx.astype(F32) * (1.0 / 160))
            mf[0, g, 0:128, :] = m.astype(BF16)
            mt = m * (2.0 / (S * D))
            if g == 0:
                mt = jnp.where(kb == 0, 0.5 * mt, mt)
                nyq = jnp.where(is_b, 0.0, jnp.where((n2 & 1) == 0, 1.0, -1.0)).astype(F32)
                mt = jnp.where(row == 8, nyq * (1.0 / (S * D)), mt)
                r16 = _iota((16, 128), 0)
                c16 = _iota((16, 128), 1)
                ext = jnp.where((r16 == 0) & (c16 < 64), jnp.where((c16 & 1) == 0, 1.0, -1.0), 0.0).astype(F32)
                mf[0, 0, 128:144, :] = ext.astype(BF16)
            mi[0, g] = mt.T.astype(BF16)

    def s_tables():
        col = _iota((16, 128), 1)
        k2 = 8 * (col & 15) + (col >> 4)

        def strip(i, carry):
            row = _iota((16, 128), 0) + 16 * i
            ga, gb = _expi_quarter(((row * k2) & 127).astype(F32) * (1.0 / 32))
            ta, tb = _expi_quarter(row.astype(F32) * (1.0 / 512))
            rs = pl.ds(pl.multiple_of(16 * i, 16), 16)
            for k1 in range(16):
                gf[0, k1, 0, rs, :] = ga.astype(BF16)
                gf[0, k1, 1, rs, :] = (gb - ga).astype(BF16)
                gf[0, k1, 2, rs, :] = (ga + gb).astype(BF16)
                if k1 < 15:
                    ga, gb = ga * ta - gb * tb, ga * tb + gb * ta
            return carry

        jax.lax.fori_loop(0, 8, strip, 0, unroll=2)

    def w_t1(b):
        for jt in range(16):
            blk = pltpu.bitcast(wraw[_tile(b), _tile(jt)].T, U32)
            for a in range(8):
                pos = 8 * (16 * a + jt)
                wt1[b][0, pos: pos + 8, :] = blk[8 * a: 8 * a + 8]
            yield

    def w_t2(b):
        z = zz()
        for m in (0, 2, 4, 6, 1, 3, 5, 7):
            wt2[m % 2][0, m // 2, _tile(b), :] = wt1[b][z, pl.ds(m, 128, stride=8), :].T
            yield

    def w_extra():
        r8 = _iota((8, S), 0)
        lane = _iota((8, 128), 1)
        e = jnp.where(r8 == 0, jnp.broadcast_to(wlast[0].astype(F32), (8, S)),
                      jnp.where(r8 == 1, jnp.broadcast_to(wlast[1].astype(F32), (8, S)), 0.0))
        v = [e[:, _tile(n)] for n in range(16)]
        for b in range(4):
            stp = 1 << b
            msk = (lane & stp) == 0
            for n in range(16):
                if n & stp:
                    continue
                lo, hi = v[n], v[n | stp]
                v[n] = jnp.where(msk, lo, pltpu.roll(hi, stp, 1))
                v[n | stp] = jnp.where(msk, pltpu.roll(lo, 128 - stp, 1), hi)
            yield
        r = _iota((8, 128), 0)
        for n in range(16):
            wex[0, n, 0] = jnp.where(r == 0, v[n], 0.0)
            wex[0, n, 1] = jnp.where(r == 0, pltpu.roll(v[n], 7, 0), 0.0)
        yield

    bias = {}

    def bias_prep():
        bias[2] = b2_ref[...].astype(F32).reshape(1, S)
        b1 = b1_ref[...].astype(F32).reshape(1, F)
        b1 = jnp.concatenate([b1, jnp.zeros((1, NFT * 128 - F), F32)], axis=1)
        for j in range(NFT):
            b1c[0, _tile(j), :] = jnp.broadcast_to(b1[:, _tile(j)], (128, 128)).T
            yield

    rstd, mean, x_done, outs = {}, {}, set(), []

    def ld(src, z, rs, n):
        return (src[z, 0, rs, _tile(n)], src[z, 1, rs, _tile(n)])

    def st(dst, rs, n, v):
        dst[0, 0, rs, _tile(n)] = v[0]
        dst[0, 1, rs, _tile(n)] = v[1]

    def x_in(tiles):
        for t in tiles:
            for j in range(5):
                XA[t][0, _tile(j), :] = xio[_tile(t), _tile(j)].T.astype(F32)
                if j == 4:
                    x_done.add(t)
                yield

    def front_vpu(tiles):
        for t in tiles:
            z = zz()
            e0s, ssq = [], None
            for rp in range(4):
                xs = [XA[t][z, 64 * n + 16 * rp: 64 * n + 16 * rp + 16, :] for n in range(10)]
                sm = [xs[n] + xs[n + 5] for n in range(5)]
                df = [xs[n] - xs[n + 5] if n % 2 == 0 else xs[n + 5] - xs[n] for n in range(5)]
                e0, e1r, e1i, e2r, e2i = _dft5(sm)
                o0, o1r, o1i, o2r, o2i = _dft5(df)
                q = (0.5 * (o0 * o0) + (e1r * e1r + e2r * e2r + o1r * o1r + o2r * o2r)
                     + (_S1 * _S1) * (e1i * e1i + o1i * o1i) + (_S2 * _S2) * (e2i * e2i + o2i * o2i))
                ssq = q if ssq is None else ssq + q
                e0s.append(e0)
                a, b = slice(16 * rp, 16 * rp + 16), slice(64 + 16 * rp, 64 + 16 * rp + 16)
                YB[t][0, 0, b, :] = o0.astype(BF16)
                for g, (va, vb) in enumerate(((o2r, o2i), (e1r, e1i), (o1r, o1i), (e2r, e2i))):
                    YB[t][0, g + 1, a, :] = va.astype(BF16)
                    YB[t][0, g + 1, b, :] = vb.astype(BF16)
                if rp < 3:
                    yield
            tot = jnp.sum(e0s[0] + e0s[1] + e0s[2] + e0s[3], axis=0, keepdims=True)
            mu10 = tot * (1.0 / 64)
            mean[t] = tot * (1.0 / D)
            e0s = [e - mu10 for e in e0s]
            q0 = e0s[0] * e0s[0] + e0s[1] * e0s[1] + e0s[2] * e0s[2] + e0s[3] * e0s[3]
            var = jnp.sum(ssq + 0.5 * q0, axis=0, keepdims=True) * (2.0 / (10 * D))
            rstd[t] = jax.lax.rsqrt(var + EPS)
            for rp in range(4):
                YB[t][0, 0, 16 * rp: 16 * rp + 16, :] = e0s[rp].astype(BF16)
            yield

    def front_mxu(b):
        z = zz(b)
        for g in range(5):
            lhs = ldb(mf, z, 0) if g == 0 else ldb(mf, z, g, slice(0, 64))
            y = _dot(lhs, jnp.concatenate([ldb(YB[4 * a + b], z, g) for a in range(4)], axis=1))
            sc_ = lambda r0, a: y[r0: r0 + 8, _tile(a)] * rstd[4 * a + b]
            for i in range(9 if g == 0 else 8):
                if i < 8:
                    xs = [(sc_(16 * i, a), sc_(16 * i + 8, a)) for a in range(4)]
                else:
                    xs = [(sc_(128, a), jnp.zeros((8, 128), F32)) for a in range(4)]
                t = _dft4(xs, -1)
                for ka in range(4):
                    st(U[g], slice(8 * i, 8 * i + 8), 4 * ka + b, _twid16(t[ka], b * ka, -1))
            yield

    def pass_f(gs):
        zt = zz(gs[0])
        cat = lambda vs: jnp.concatenate(vs, axis=0) if len(vs) > 1 else vs[0]
        for ka in range(4):
            for par in range(2):
                xs = []
                for b in range(4):
                    pr = [ld(U[g], zz(par), slice(0, _ROWS[g]), 4 * ka + b) for g in gs]
                    xs.append((cat([p[0] for p in pr]), cat([p[1] for p in pr])))
                for h, (ur, ui) in enumerate(_dft4_half(xs, -1, par)):
                    k1 = ka + 4 * (par + 2 * h)
                    p1 = _dot((ur + ui).astype(BF16), ldb(gf, zt, k1, 0))
                    p2 = _dot(ur.astype(BF16), ldb(gf, zt, k1, 1))
                    p3 = _dot(ui.astype(BF16), ldb(gf, zt, k1, 2))
                    xr, xi = p1 - p3, p1 + p2
                    r0 = 0
                    for g in gs:
                        st(XS[g], slice(0, _ROWS[g]), k1, (xr[r0: r0 + _ROWS[g]], xi[r0: r0 + _ROWS[g]]))
                        r0 += _ROWS[g]
                yield

    def w_rows(z, a, g, k1):
        parts = []
        for res in _RES[g]:
            blk = wt2[(k1 // 2) % 2][z, k1 // 4, pl.ds(320 * a + res, 32, stride=10), :]
            blk = (blk << 16) if k1 % 2 == 0 else (blk & jnp.uint32(0xFFFF0000))
            parts.append(pltpu.bitcast(blk, F32))
        if g == 0:
            parts.append(jnp.concatenate([wex[z, k1, a], jnp.zeros((8, 128), F32)], axis=0))
        return parts

    def pass_i(g):
        z = zz(g + 3)
        rs = slice(0, _ROWS[g])
        for ka in range(4):
            vs = []
            for kb in range(4):
                k1 = ka + 4 * kb
                xr, xi = ld(XS[g], z, rs, k1)
                wr, wi = [jnp.concatenate(w_rows(z, a, g, k1), axis=0) for a in range(2)]
                yr = xr * wr - xi * wi
                yi = xr * wi + xi * wr
                q1, q2, q3 = [jax.lax.dot_general(v.astype(BF16), ldb(gf, z, k1, j), NT, preferred_element_type=F32)
                              for j, v in enumerate((yr + yi, yi, yr))]
                vs.append((q1 + q2, q1 - q3))
                if kb == 1:
                    yield
            t = _dft4(vs, +1)
            for b in range(4):
                st(V[g], rs, 4 * ka + b, _twid16(t[b], b * ka, +1))
            yield

    def pass_b(g, bs=range(4)):
        for b in bs:
            z = zz(b)
            rhs = [[] for _ in range(4)]
            for i in range(8):
                rs = slice(8 * i, 8 * i + 8)
                y = _dft4([ld(V[g], z, rs, 4 * ka + b) for ka in range(4)], +1)
                if g == 0 and i == 0:
                    r8 = _iota((8, 128), 0)
                    ex = _dft4([ld(V[0], z, slice(64, 72), 4 * ka + b) for ka in range(4)], +1)
                    y = [(y[a][0], jnp.where(r8 == 0, ex[a][0], y[a][1])) for a in range(4)]
                for a in range(4):
                    rhs[a] += [y[a][0], y[a][1]]
            yield
            for a in range(4):
                Q[g][b][0, a] = _dot(ldb(mi, z, g), jnp.concatenate(rhs[a], axis=0).astype(BF16))
            yield

    def back_vpu(tiles):
        for t in tiles:
            z = zz(1)
            qa, qb = t // 4, t % 4
            q = lambda g, rs: Q[g][qb][z, qa, rs, :]
            q0 = [q(0, slice(8 * rp, 8 * rp + 8)) for rp in range(8)]
            qs = ((q0[0] + q0[1]) + (q0[2] + q0[3])) + ((q0[4] + q0[5]) + (q0[6] + q0[7]))
            mu = mean[t] + jnp.sum(qs, axis=0, keepdims=True) * (10.0 / D)
            mean[t] = mu
            s2 = [None, None]
            for rp in range(8):
                a, b = slice(8 * rp, 8 * rp + 8), slice(64 + 8 * rp, 64 + 8 * rp + 8)
                e = _dft5_t(q0[rp] - mu, q(2, a), q(2, b), q(4, a), q(4, b))
                o = _dft5_t(q(0, b), q(3, a), q(3, b), q(1, a), q(1, b))
                for n in range(5):
                    lo = slice(64 * n + 8 * rp, 64 * n + 8 * rp + 8)
                    hi = slice(64 * (n + 5) + 8 * rp, 64 * (n + 5) + 8 * rp + 8)
                    if n % 2 == 0:
                        ylo, yhi = e[n] + o[n], e[n] - o[n]
                    else:
                        ylo, yhi = e[n] - o[n], e[n] + o[n]
                    xlo = XA[t][z, lo, :] + ylo
                    xhi = XA[t][z, hi, :] + yhi
                    XB[t][0, lo, :] = xlo
                    XB[t][0, hi, :] = xhi
                    s2[0] = xlo * xlo if s2[0] is None else s2[0] + xlo * xlo
                    s2[1] = xhi * xhi if s2[1] is None else s2[1] + xhi * xhi
                if rp % 2 == 1:
                    yield
            var = jnp.sum(s2[0] + s2[1], axis=0, keepdims=True) * (1.0 / D)
            r1 = jax.lax.rsqrt(var + EPS)
            r2 = jax.lax.rsqrt(var * r1 * r1 + EPS)
            rr = r1 * r2
            for i in range(D // 16):
                HB[t][0, 16 * i: 16 * i + 16, :] = (XB[t][z, 16 * i: 16 * i + 16, :] * rr).astype(BF16)
            yield

    def act(get, off, w, zi):
        z = zz(zi)
        for r0 in range(0, w, 128):
            r1 = min(r0 + 128, w)
            j = (off + r0) // 128
            for i in range(5):
                parts = []
                for q in range(r0, r1, 32):
                    u = get(q, q + 32, i) + b1c[z, off + q: off + q + 32, :]
                    parts.append(_gelu(u))
                g = jnp.concatenate(parts, axis=0).astype(BF16).T
                GB[j][0, 64 * i: 64 * i + 64, 0: r1 - r0] = pltpu.bitcast(g, U32)
                yield

    def mm1_dot(off, w, zi):
        z = zz(zi)
        rhs = jnp.concatenate([ldb(HB[t], z) for t in range(NTT)], axis=1)
        u = jax.lax.dot_general(w1t[off: off + w, :], rhs, NT, preferred_element_type=F32)
        return lambda r0, r1, i: u[r0:r1, _tile(i)]

    def mm1_step(tiles, first):
        z = zz()
        lhs = jnp.concatenate([w1t[0:W1C, _tile(t)] for t in tiles], axis=1)
        for i in range(5):
            rhs = jnp.concatenate([ldb(HB[t], z, slice(64 * i, 64 * i + 64)) for t in tiles], axis=1)
            part = jax.lax.dot_general(lhs, rhs, NT, preferred_element_type=F32)
            ACC[i][0] = part if first else ACC[i][z] + part
            yield

    def mm2(c, tiles, d0=0, d1=D):
        z = zz(c % 8)
        rs = slice(d0 // 2, d1 // 2)
        parts = [GB[j][z, rs, :] for j in range(NFT - 1)] + [GB[NFT - 1][z, rs, 0: F % 128]]
        y = _dot(jnp.concatenate([pltpu.bitcast(p, BF16) for p in parts], axis=1),
                 jnp.concatenate([w2[:, _tile(t)] for t in tiles], axis=1))
        return [XB[t][zz(2), d0:d1, :] + (y[:, _tile(i)] + (bias[2][:, _tile(t)] + mean[t]))
                for i, t in enumerate(tiles)]

    chain = itertools.chain
    P = _PAIRS
    d_tables()
    U[0][0, :, 72:80, :] = jnp.zeros((2, 8, S), F32)
    s_tables()

    pend_v, fv_done, fm_done = [], [], []
    for c, seg in enumerate(_XSEG):
        last = c == len(_XSEG) - 1
        for t in seg:
            x_copy(t).wait()
        if c == 0:
            z_copy.wait()
            zpool.extend(sc["zs"][0, i] for i in range(NZ))
        if last:
            for cp in small:
                cp.wait()
        ready = [b for b in range(3) if b not in fm_done and all(4 * a + b in fv_done for a in range(4))]
        fm_done += ready
        cand = pend_v + seg
        fv, pend_v = (cand, []) if last else (cand[:-1], cand[-1:])
        fv_done += fv
        xg = x_in(seg)

        def fv_gen(tiles, xg=xg):
            for t in tiles:
                while t not in x_done:
                    next(xg)
                yield from front_vpu([t])

        _weave((xg, 5 * len(seg)), (fv_gen(fv), 4 * len(fv) + 2),
               (chain(*[front_mxu(b) for b in ready]) if ready else None, 5), (w_extra() if last else None, 5))
    _weave((chain(*[front_mxu(b) for b in range(4) if b not in fm_done]), 5))

    for layer in range(2):
        lay[0] = layer
        if layer == 0:
            for gs in ((0, 1), (2, 3), (4,)):
                for r in gs:
                    for cp in w_copies[r]:
                        cp.wait()
                _weave((pass_f(gs), 8), (chain(*([w_t1(r) for r in gs] + [w_t2(r) for r in gs])), 24 * len(gs)))
        else:
            fence()
            _weave((pass_f((0, 1, 2, 3, 4)), 8))
        for g in range(5):
            _weave((pass_i(g), 8))
        _weave((chain(*[pass_b(g, [0]) for g in range(4)]), 8))
        if layer == 0:
            w1_copy(0).wait()
        else:
            fence()
        ball = lambda b: chain(*[pass_b(g, [b]) for g in range(5)])
        _weave((pass_b(4, [0]), 2))
        _weave((ball(1), 10), (back_vpu(P[0]), 10))
        _weave((ball(2), 10), (back_vpu(P[1]), 10))
        _weave((ball(3), 10), (back_vpu(P[2]), 10))
        _weave((mm1_step(P[0] + P[1], True), 5), (back_vpu(P[3] + P[4]), 20))
        _weave((mm1_step(P[2] + P[3], False), 5), (back_vpu(P[5] + P[6] + P[7]), 30))
        _weave((mm1_step(P[4] + P[5], False), 5))
        _weave((mm1_step(P[6] + P[7], False), 5), (bias_prep() if layer == 0 else None, NFT))
        if layer == 0:
            for i in range(1, NW1):
                w1_copy(i).wait()
        za = zz(1)
        pend = (lambda r0, r1, i: ACC[i][za, r0:r1, :], 0, W1C, 0)
        off = W1C
        for i, w in enumerate(W1S):
            if layer == 0 and i == len(W1S) - 1:
                for cp in [w2_copy(j) for j in range(NW2)] + seps:
                    cp.wait()
            cur = (mm1_dot(off, w, i + 1), off, w, i + 1)
            _weave((act(*pend), 1))
            pend = cur
            off += w
        _weave((act(*pend), 1))
        chunks = [P[0] + P[1], P[2] + P[3], P[4] + P[5], P[6], P[7]]
        nch = len(chunks)
        if layer == 0:
            for c in range(nch + 1):
                if c < nch:
                    for t, v in zip(chunks[c], mm2(c, chunks[c])):
                        XA[t][0] = v
                lay[0] = 1
                if c == nch:
                    _weave((front_mxu(2), 5), (front_vpu(chunks[c - 1]), 8))
                    _weave((front_mxu(3), 5))
                elif c >= 1:
                    _weave((front_vpu(chunks[c - 1]), 8))
                    if c <= 2:
                        _weave((front_mxu(c - 1), 5))
                lay[0] = 0
        else:
            jobs = [(c, chunks[c], 0, D) for c in range(nch - 1)]
            jobs += [(nch - 1, chunks[-1], 0, DS), (nch, chunks[-1], DS, D)]
            prev = None
            for n, job in enumerate(jobs + [None]):
                cur = (job, mm2(*job)) if job is not None else None
                if prev is not None:
                    (_, tiles, d0, d1), vals = prev
                    for i, (t, v) in enumerate(zip(tiles, vals)):
                        xio[_tile(t), d0:d1] = v.astype(BF16).T
                        outs.append(o_copy(t, d0, d1, NTT + i if d0 else None))
                        outs[-1].start()
                    if n in (nch - 2, nch):
                        fence()
                prev = cur

    for cp in outs:
        cp.wait()


@jax.jit
def pallas_interleave_layers__spectral_gfnet__mixer_token_mlp__prompt_kernel(A_x, A_w_r, A_w_i, B_x, B_w1, B_b1, B_w2, B_b2):
    del B_x
    any_spec = pl.BlockSpec(memory_space=pl.ANY)
    return pl.pallas_call(
        _kernel,
        out_shape=jax.ShapeDtypeStruct((1, S, D), BF16),
        in_specs=[any_spec] * 7,
        out_specs=any_spec,
        scratch_shapes=jax.tree_util.tree_leaves(_scratch(), is_leaf=_is_leaf),
        compiler_params=pltpu.CompilerParams(vmem_limit_bytes=120 * 1024 * 1024, disable_semaphore_checks=True),
    )(A_x, A_w_r.T, A_w_i.T, B_w1.T, B_b1, B_w2, B_b2)
```

```python
import itertools
import math

import jax
import jax.numpy as jnp
import jax.experimental.pallas as pl
import jax.experimental.pallas.tpu as pltpu

S = 2048
D = 640
F = 1728
EPS = 1e-5
F32 = jnp.float32
BF16 = jnp.bfloat16
U32 = jnp.uint32
NT = (((1,), (1,)), ((), ()))

_C1, _C2 = math.cos(2 * math.pi / 5), math.cos(4 * math.pi / 5)
_S1, _S2 = math.sin(2 * math.pi / 5), math.sin(4 * math.pi / 5)
_KN = (_C1 - _C2) / 2
_RES = ((0, 5), (1, 9), (2, 8), (3, 7), (4, 6))
_BASE = (None, 9, 2, 7, 4)
_SC = (None, _S2, _S1, _S1, _S2)
_ROWS = (80, 64, 64, 64, 64)

W1C = 640
W1S = (384, 384, 320)
NW1 = -(-F // W1C)
W2C = 216
NW2 = F // W2C
NFT = -(-F // 128)
NTT = S // 128
NZ = 16
DS = 512
_PAIRS = [(b + 8 * h, b + 8 * h + 4) for b in range(4) for h in range(2)]
_XSEG = [[0, 4, 8, 12], [1, 5, 9, 13], [2, 6], [10, 14], [3, 7], [11, 15]]


def _dft5(a):
    a1 = a[1] + a[4]
    b1 = a[1] - a[4]
    a2 = a[2] + a[3]
    b2 = a[2] - a[3]
    t = a1 + a2
    y0 = a[0] + t
    m = a[0] - 0.25 * t
    n = _KN * (a1 - a2)
    return y0, m + n, b1 + (_S2 / _S1) * b2, m - n, b1 - (_S1 / _S2) * b2


def _dft5_t(y0, y1r, y1i, y2r, y2i):
    gm = y1r + y2r
    gn = _KN * (y1r - y2r)
    a0 = y0 + gm
    gt = y0 - 0.25 * gm
    ga1 = gt + gn
    ga2 = gt - gn
    gb1 = y1i + y2i
    gb2 = (_S2 / _S1) * y1i - (_S1 / _S2) * y2i
    return [a0, ga1 + gb1, ga2 + gb2, ga2 - gb2, ga1 - gb1]


def _dft4_half(x, sign, par):
    (ar, ai), (br, bi), (cr, ci), (dr, di) = x
    if par == 0:
        t0r, t0i, t2r, t2i = ar + cr, ai + ci, br + dr, bi + di
        return [(t0r + t2r, t0i + t2i), (t0r - t2r, t0i - t2i)]
    t1r, t1i, t3r, t3i = ar - cr, ai - ci, br - dr, bi - di
    p, m = (t1r + t3i, t1i - t3r), (t1r - t3i, t1i + t3r)
    return [p, m] if sign < 0 else [m, p]


def _dft4(x, sign):
    y0, y2 = _dft4_half(x, sign, 0)
    y1, y3 = _dft4_half(x, sign, 1)
    return [y0, y1, y2, y3]


def _twid16(v, e, sign):
    r, i = v
    e = e % 16
    if e == 0:
        return v
    h = math.sqrt(0.5)
    if e == 4:
        return (-i, r) if sign > 0 else (i, -r)
    if e == 2:
        return (h * (r - i), h * (r + i)) if sign > 0 else (h * (r + i), h * (i - r))
    if e == 6:
        return (-h * (r + i), h * (r - i)) if sign > 0 else (h * (i - r), -h * (r + i))
    c = math.cos(2 * math.pi * e / 16)
    s = sign * math.sin(2 * math.pi * e / 16)
    return (c * r - s * i, s * r + c * i)


def _iota(shape, dim):
    return jax.lax.broadcasted_iota(jnp.int32, shape, dim)


def _cos_quarter(t):
    q = jnp.floor(t + 0.5)
    x = (t - q) * (math.pi / 2)
    x2 = x * x
    c = 1.0 + x2 * (-1.0 / 2 + x2 * (1.0 / 24 + x2 * (-1.0 / 720 + x2 * (1.0 / 40320))))
    s = x * (1.0 + x2 * (-1.0 / 6 + x2 * (1.0 / 120 + x2 * (-1.0 / 5040 + x2 * (1.0 / 362880)))))
    qi = q.astype(jnp.int32)
    v = jnp.where((qi & 1) == 1, s, c)
    return jnp.where(((qi + 1) & 2) == 2, -v, v)


def _expi_quarter(t):
    q = jnp.floor(t + 0.5)
    x = (t - q) * (math.pi / 2)
    x2 = x * x
    c = 1.0 + x2 * (-1.0 / 2 + x2 * (1.0 / 24 + x2 * (-1.0 / 720 + x2 * (1.0 / 40320))))
    s = x * (1.0 + x2 * (-1.0 / 6 + x2 * (1.0 / 120 + x2 * (-1.0 / 5040 + x2 * (1.0 / 362880)))))
    qi = q.astype(jnp.int32)
    odd = (qi & 1) == 1
    u = jnp.where(odd, s, c)
    v = jnp.where(odd, c, s)
    return jnp.where(((qi + 1) & 2) == 2, -u, u), jnp.where((qi & 2) == 2, v, -v)


def _gelu(x):
    c = math.sqrt(2 / math.pi)
    h = 0.5 * x
    return h + h * jnp.tanh(x * (c + (c * 0.044715) * (x * x)))


def _dot(a, b):
    return jnp.dot(a, b, preferred_element_type=F32)


def _tile(n):
    return slice(128 * n, 128 * n + 128)


def _weave(*streams):
    live = [[g, n, 0] for g, n in streams if g is not None]
    while live:
        cur = min(live, key=lambda e: (e[2] + 0.5) / e[1])
        try:
            next(cur[0])
            cur[2] += 1
        except StopIteration:
            live.remove(cur)


def _scratch():
    v = lambda shape, dt: pltpu.VMEM((1,) + shape, dt)
    return dict(
        xio=pltpu.VMEM((S, D), BF16),
        wraw=pltpu.VMEM((640, S), BF16),
        wlast=pltpu.VMEM((4, 1, S), BF16),
        w1t=pltpu.VMEM((F, S), BF16),
        w2=pltpu.VMEM((F, S), BF16),
        b1v=pltpu.VMEM((F,), BF16),
        b2v=pltpu.VMEM((S,), BF16),
        wt1=[v((S // 2, 128), U32) for _ in range(5)],
        wt2=[v((4, 640, 128), U32) for _ in range(2)],
        wex=v((16, 2, 8, 128), F32),
        b1c=v((NFT * 128, 128), F32),
        ACC=[v((W1C, 128), F32) for _ in range(5)],
        XA=[v((D, 128), F32) for _ in range(NTT)],
        XB=[v((D, 128), F32) for _ in range(NTT)],
        YB=[v((5, 128, 128), BF16) for _ in range(NTT)],
        U=[v((2, r, S), F32) for r in _ROWS],
        XS=[v((2, r, S), F32) for r in _ROWS],
        V=[v((2, r, S), F32) for r in _ROWS],
        Q=[[v((4, 128, 128), F32) for _ in range(4)] for _ in range(5)],
        HB=[v((D, 128), BF16) for _ in range(NTT)],
        GB=[v((D // 2, 128), U32) for _ in range(NFT)],
        gf=v((16, 3, 128, 128), BF16),
        mf=v((5, 144, 128), BF16),
        mi=v((5, 128, 128), BF16),
        sem_x=pltpu.SemaphoreType.DMA((NTT,)),
        sem_w=pltpu.SemaphoreType.DMA((12,)),
        sem_w1=pltpu.SemaphoreType.DMA((NW1,)),
        sem_w2=pltpu.SemaphoreType.DMA((NW2,)),
        sem_o=pltpu.SemaphoreType.DMA((NTT + 2,)),
        zv=pltpu.VMEM((8, 128), jnp.int32),
        zs=pltpu.SMEM((8, 128), jnp.int32),
        sem_z=pltpu.SemaphoreType.DMA,
        sem_f=pltpu.SemaphoreType.REGULAR,
    )


def _is_leaf(x):
    return not isinstance(x, (dict, list))


def _kernel(x_hbm, wr_hbm, wi_hbm, w1t_hbm, b1_hbm, w2_hbm, b2_hbm, o_hbm, *scratch):
    sc = jax.tree_util.tree_unflatten(jax.tree_util.tree_structure(_scratch(), is_leaf=_is_leaf), scratch)
    xio, wraw, wlast, w1t, w2, b1_ref, b2_ref = (sc[k] for k in ("xio", "wraw", "wlast", "w1t", "w2", "b1v", "b2v"))
    wt1, wt2, wex, b1c, ACC = (sc[k] for k in ("wt1", "wt2", "wex", "b1c", "ACC"))
    XA, XB, YB, U, XS, V, Q, HB, GB = (sc[k] for k in ("XA", "XB", "YB", "U", "XS", "V", "Q", "HB", "GB"))
    gf, mf, mi = (sc[k] for k in ("gf", "mf", "mi"))
    sem_x, sem_w, sem_w1, sem_w2, sem_o = (sc[k] for k in ("sem_x", "sem_w", "sem_w1", "sem_w2", "sem_o"))

    def x_copy(t):
        return pltpu.make_async_copy(x_hbm.at[0, pl.ds(t * 128, 128), :], xio.at[pl.ds(t * 128, 128), :], sem_x.at[t])

    def o_copy(t, d0=0, d1=D, k=None):
        return pltpu.make_async_copy(xio.at[pl.ds(t * 128, 128), pl.ds(d0, d1 - d0)],
                                     o_hbm.at[0, pl.ds(t * 128, 128), pl.ds(d0, d1 - d0)],
                                     sem_o.at[t if k is None else k])

    w_parts = [[(wr_hbm, 0, 0, 128)], [(wr_hbm, 128, 128, 128)], [(wr_hbm, 256, 256, 64), (wi_hbm, 0, 320, 64)],
               [(wi_hbm, 64, 384, 128)], [(wi_hbm, 192, 512, 128)]]
    w_copies, n = [], 0
    for blk in w_parts:
        cur = []
        for (src, s0, d0, rows) in blk:
            cur.append(pltpu.make_async_copy(src.at[pl.ds(s0, rows), :], wraw.at[pl.ds(d0, rows), :], sem_w.at[n]))
            n += 1
        w_copies.append(cur)
    small = []
    for a, src in enumerate((wr_hbm, wi_hbm)):
        small.append(pltpu.make_async_copy(src.at[pl.ds(320, 1), :], wlast.at[a], sem_w.at[n]))
        n += 1
    for src, dst in ((b1_hbm, b1_ref), (b2_hbm, b2_ref)):
        small.append(pltpu.make_async_copy(src, dst, sem_w.at[n]))
        n += 1

    def w1_copy(i):
        rows = min(W1C, F - i * W1C)
        return pltpu.make_async_copy(w1t_hbm.at[pl.ds(i * W1C, rows), :], w1t.at[pl.ds(i * W1C, rows), :], sem_w1.at[i])

    def w2_copy(i):
        return pltpu.make_async_copy(w2_hbm.at[pl.ds(i * W2C, W2C), :], w2.at[pl.ds(i * W2C, W2C), :], sem_w2.at[i])

    seps = [pltpu.make_async_copy(wr_hbm.at[pl.ds(320, 1), :], wlast.at[2 + a], sem_w.at[n + a]) for a in range(2)]

    sc["zv"][...] = jnp.zeros((8, 128), jnp.int32)
    z_copy = pltpu.make_async_copy(sc["zv"], sc["zs"], sc["sem_z"])
    z_copy.start()
    for cp in [x_copy(t) for seg in _XSEG for t in seg] + small + [cp for blk in w_copies for cp in blk] + seps[:1]:
        cp.start()
    for cp in [w1_copy(i) for i in range(NW1)] + seps[1:] + [w2_copy(i) for i in range(NW2)]:
        cp.start(priority=1)

    zpool = []
    lay = [0]

    def zz(i=0):
        return zpool[8 * lay[0] + i]

    def ldb(ref, z, *idx):
        return pltpu.bitcast(ref.bitcast(U32)[(z,) + idx], BF16)

    def fence():
        pl.semaphore_signal(sc["sem_f"], 1)
        pl.semaphore_wait(sc["sem_f"], 1)

    def d_tables():
        row = _iota((128, 128), 0)
        col = _iota((128, 128), 1)
        n2 = col & 63
        is_b = col >= 64
        is_im = (row & 8) == 8
        rr = ((row >> 4) << 3) | (row & 7)
        j = rr & 31
        second = rr >= 32
        for g in range(5):
            ra, rb = _RES[g]
            kb = jnp.where(second, rb, ra) + 10 * j
            idx = kb * n2
            if g == 0:
                idx = idx + jnp.where(is_im, 160, 0)
                amp = jnp.where(second == is_b, 1.0, 0.0).astype(F32)
            else:
                idx = idx + jnp.where(is_im != is_b, 160, 0)
                sg = jnp.where((rb == _BASE[g]) == second, 1.0, -1.0).astype(F32)
                amp = jnp.where(is_b, jnp.where(is_im, -sg * _SC[g], sg * _SC[g]), 1.0).astype(F32)
            m = amp * _cos_quarter(idx.astype(F32) * (1.0 / 160))
            mf[0, g, 0:128, :] = m.astype(BF16)
            mt = m * (2.0 / (S * D))
            if g == 0:
                mt = jnp.where(kb == 0, 0.5 * mt, mt)
                nyq = jnp.where(is_b, 0.0, jnp.where((n2 & 1) == 0, 1.0, -1.0)).astype(F32)
                mt = jnp.where(row == 8, nyq * (1.0 / (S * D)), mt)
                r16 = _iota((16, 128), 0)
                c16 = _iota((16, 128), 1)
                ext = jnp.where((r16 == 0) & (c16 < 64), jnp.where((c16 & 1) == 0, 1.0, -1.0), 0.0).astype(F32)
                mf[0, 0, 128:144, :] = ext.astype(BF16)
            else:
                mf[0, g, 128:144, :] = jnp.zeros((16, 128), BF16)
            mi[0, g] = mt.T.astype(BF16)

    def s_tables():
        col = _iota((16, 128), 1)
        k2 = 8 * (col & 15) + (col >> 4)

        def strip(i, carry):
            row = _iota((16, 128), 0) + 16 * i
            ga, gb = _expi_quarter(((row * k2) & 127).astype(F32) * (1.0 / 32))
            ta, tb = _expi_quarter(row.astype(F32) * (1.0 / 512))
            rs = pl.ds(pl.multiple_of(16 * i, 16), 16)
            for k1 in range(16):
                gf[0, k1, 0, rs, :] = ga.astype(BF16)
                gf[0, k1, 1, rs, :] = (gb - ga).astype(BF16)
                gf[0, k1, 2, rs, :] = (ga + gb).astype(BF16)
                if k1 < 15:
                    ga, gb = ga * ta - gb * tb, ga * tb + gb * ta
            return carry

        jax.lax.fori_loop(0, 8, strip, 0, unroll=2)

    def w_t1(b):
        for jt in range(16):
            blk = pltpu.bitcast(wraw[_tile(b), _tile(jt)].T, U32)
            for a in range(8):
                pos = 8 * (16 * a + jt)
                wt1[b][0, pos: pos + 8, :] = blk[8 * a: 8 * a + 8]
            yield

    def w_t2(b):
        z = zz()
        for m in (0, 2, 4, 6, 1, 3, 5, 7):
            wt2[m % 2][0, m // 2, _tile(b), :] = wt1[b][z, pl.ds(m, 128, stride=8), :].T
            yield

    def w_extra():
        r8 = _iota((8, S), 0)
        lane = _iota((8, 128), 1)
        e = jnp.where(r8 == 0, jnp.broadcast_to(wlast[0].astype(F32), (8, S)),
                      jnp.where(r8 == 1, jnp.broadcast_to(wlast[1].astype(F32), (8, S)), 0.0))
        v = [e[:, _tile(n)] for n in range(16)]
        for b in range(4):
            stp = 1 << b
            msk = (lane & stp) == 0
            for n in range(16):
                if n & stp:
                    continue
                lo, hi = v[n], v[n | stp]
                v[n] = jnp.where(msk, lo, pltpu.roll(hi, stp, 1))
                v[n | stp] = jnp.where(msk, pltpu.roll(lo, 128 - stp, 1), hi)
            yield
        r = _iota((8, 128), 0)
        for n in range(16):
            wex[0, n, 0] = jnp.where(r == 0, v[n], 0.0)
            wex[0, n, 1] = jnp.where(r == 0, pltpu.roll(v[n], 7, 0), 0.0)
        yield

    bias = {}

    def bias_prep():
        bias[2] = b2_ref[...].astype(F32).reshape(1, S)
        b1 = b1_ref[...].astype(F32).reshape(1, F)
        b1 = jnp.concatenate([b1, jnp.zeros((1, NFT * 128 - F), F32)], axis=1)
        for j in range(NFT):
            b1c[0, _tile(j), :] = jnp.broadcast_to(b1[:, _tile(j)], (128, 128)).T
            yield

    rstd, mean, x_done, outs = {}, {}, set(), []

    def ld(src, z, rs, n):
        return (src[z, 0, rs, _tile(n)], src[z, 1, rs, _tile(n)])

    def st(dst, rs, n, v):
        dst[0, 0, rs, _tile(n)] = v[0]
        dst[0, 1, rs, _tile(n)] = v[1]

    def x_in(tiles):
        for t in tiles:
            for j in range(5):
                XA[t][0, _tile(j), :] = xio[_tile(t), _tile(j)].T.astype(F32)
                if j == 4:
                    x_done.add(t)
                yield

    def front_vpu(tiles):
        for t in tiles:
            z = zz()
            e0s, ssq = [], None
            for rp in range(4):
                xs = [XA[t][z, 64 * n + 16 * rp: 64 * n + 16 * rp + 16, :] for n in range(10)]
                sm = [xs[n] + xs[n + 5] for n in range(5)]
                df = [xs[n] - xs[n + 5] if n % 2 == 0 else xs[n + 5] - xs[n] for n in range(5)]
                e0, e1r, e1i, e2r, e2i = _dft5(sm)
                o0, o1r, o1i, o2r, o2i = _dft5(df)
                q = (0.5 * (o0 * o0) + (e1r * e1r + e2r * e2r + o1r * o1r + o2r * o2r)
                     + (_S1 * _S1) * (e1i * e1i + o1i * o1i) + (_S2 * _S2) * (e2i * e2i + o2i * o2i))
                ssq = q if ssq is None else ssq + q
                e0s.append(e0)
                a, b = slice(16 * rp, 16 * rp + 16), slice(64 + 16 * rp, 64 + 16 * rp + 16)
                YB[t][0, 0, b, :] = o0.astype(BF16)
                for g, (va, vb) in enumerate(((o2r, o2i), (e1r, e1i), (o1r, o1i), (e2r, e2i))):
                    YB[t][0, g + 1, a, :] = va.astype(BF16)
                    YB[t][0, g + 1, b, :] = vb.astype(BF16)
                if rp < 3:
                    yield
            tot = jnp.sum(e0s[0] + e0s[1] + e0s[2] + e0s[3], axis=0, keepdims=True)
            mu10 = tot * (1.0 / 64)
            mean[t] = tot * (1.0 / D)
            e0s = [e - mu10 for e in e0s]
            q0 = e0s[0] * e0s[0] + e0s[1] * e0s[1] + e0s[2] * e0s[2] + e0s[3] * e0s[3]
            var = jnp.sum(ssq + 0.5 * q0, axis=0, keepdims=True) * (2.0 / (10 * D))
            rstd[t] = jax.lax.rsqrt(var + EPS)
            for rp in range(4):
                YB[t][0, 0, 16 * rp: 16 * rp + 16, :] = e0s[rp].astype(BF16)
            yield

    def front_mxu(b):
        z = zz(b)
        for g in range(5):
            lhs = ldb(mf, z, 0) if g == 0 else ldb(mf, z, g, slice(0, 64))
            y = _dot(lhs, jnp.concatenate([ldb(YB[4 * a + b], z, g) for a in range(4)], axis=1))
            sc_ = lambda r0, a: y[r0: r0 + 8, _tile(a)] * rstd[4 * a + b]
            for i in range(9 if g == 0 else 8):
                if i < 8:
                    xs = [(sc_(16 * i, a), sc_(16 * i + 8, a)) for a in range(4)]
                else:
                    xs = [(sc_(128, a), jnp.zeros((8, 128), F32)) for a in range(4)]
                t = _dft4(xs, -1)
                for ka in range(4):
                    st(U[g], slice(8 * i, 8 * i + 8), 4 * ka + b, _twid16(t[ka], b * ka, -1))
            yield

    def pass_f(gs):
        zt = zz(gs[0])
        cat = lambda vs: jnp.concatenate(vs, axis=0) if len(vs) > 1 else vs[0]
        for ka in range(4):
            for par in range(2):
                xs = []
                for b in range(4):
                    pr = [ld(U[g], zz(par), slice(0, _ROWS[g]), 4 * ka + b) for g in gs]
                    xs.append((cat([p[0] for p in pr]), cat([p[1] for p in pr])))
                for h, (ur, ui) in enumerate(_dft4_half(xs, -1, par)):
                    k1 = ka + 4 * (par + 2 * h)
                    p1 = _dot((ur + ui).astype(BF16), ldb(gf, zt, k1, 0))
                    p2 = _dot(ur.astype(BF16), ldb(gf, zt, k1, 1))
                    p3 = _dot(ui.astype(BF16), ldb(gf, zt, k1, 2))
                    xr, xi = p1 - p3, p1 + p2
                    r0 = 0
                    for g in gs:
                        st(XS[g], slice(0, _ROWS[g]), k1, (xr[r0: r0 + _ROWS[g]], xi[r0: r0 + _ROWS[g]]))
                        r0 += _ROWS[g]
                yield

    def w_rows(z, a, g, k1):
        parts = []
        for res in _RES[g]:
            blk = wt2[(k1 // 2) % 2][z, k1 // 4, pl.ds(320 * a + res, 32, stride=10), :]
            blk = (blk << 16) if k1 % 2 == 0 else (blk & jnp.uint32(0xFFFF0000))
            parts.append(pltpu.bitcast(blk, F32))
        if g == 0:
            parts.append(jnp.concatenate([wex[z, k1, a], jnp.zeros((8, 128), F32)], axis=0))
        return parts

    def pass_i(g):
        z = zz(g + 3)
        rs = slice(0, _ROWS[g])
        for ka in range(4):
            vs = []
            for kb in range(4):
                k1 = ka + 4 * kb
                xr, xi = ld(XS[g], z, rs, k1)
                wr, wi = [jnp.concatenate(w_rows(z, a, g, k1), axis=0) for a in range(2)]
                yr = xr * wr - xi * wi
                yi = xr * wi + xi * wr
                q1, q2, q3 = [jax.lax.dot_general(v.astype(BF16), ldb(gf, z, k1, j), NT, preferred_element_type=F32)
                              for j, v in enumerate((yr + yi, yi, yr))]
                vs.append((q1 + q2, q1 - q3))
                if kb == 1:
                    yield
            t = _dft4(vs, +1)
            for b in range(4):
                st(V[g], rs, 4 * ka + b, _twid16(t[b], b * ka, +1))
            yield

    def pass_b(g, bs=range(4)):
        for b in bs:
            z = zz(b)
            rhs = [[] for _ in range(4)]
            for i in range(8):
                rs = slice(8 * i, 8 * i + 8)
                y = _dft4([ld(V[g], z, rs, 4 * ka + b) for ka in range(4)], +1)
                if g == 0 and i == 0:
                    r8 = _iota((8, 128), 0)
                    ex = _dft4([ld(V[0], z, slice(64, 72), 4 * ka + b) for ka in range(4)], +1)
                    y = [(y[a][0], jnp.where(r8 == 0, ex[a][0], y[a][1])) for a in range(4)]
                for a in range(4):
                    rhs[a] += [y[a][0], y[a][1]]
            yield
            for a in range(4):
                Q[g][b][0, a] = _dot(ldb(mi, z, g), jnp.concatenate(rhs[a], axis=0).astype(BF16))
            yield

    def back_vpu(tiles):
        for t in tiles:
            z = zz(1)
            qa, qb = t // 4, t % 4
            q = lambda g, rs: Q[g][qb][z, qa, rs, :]
            q0 = [q(0, slice(8 * rp, 8 * rp + 8)) for rp in range(8)]
            qs = ((q0[0] + q0[1]) + (q0[2] + q0[3])) + ((q0[4] + q0[5]) + (q0[6] + q0[7]))
            mu = mean[t] + jnp.sum(qs, axis=0, keepdims=True) * (10.0 / D)
            mean[t] = mu
            s2 = [None, None]
            for rp in range(8):
                a, b = slice(8 * rp, 8 * rp + 8), slice(64 + 8 * rp, 64 + 8 * rp + 8)
                e = _dft5_t(q0[rp] - mu, q(2, a), q(2, b), q(4, a), q(4, b))
                o = _dft5_t(q(0, b), q(3, a), q(3, b), q(1, a), q(1, b))
                for n in range(5):
                    lo = slice(64 * n + 8 * rp, 64 * n + 8 * rp + 8)
                    hi = slice(64 * (n + 5) + 8 * rp, 64 * (n + 5) + 8 * rp + 8)
                    if n % 2 == 0:
                        ylo, yhi = e[n] + o[n], e[n] - o[n]
                    else:
                        ylo, yhi = e[n] - o[n], e[n] + o[n]
                    xlo = XA[t][z, lo, :] + ylo
                    xhi = XA[t][z, hi, :] + yhi
                    XB[t][0, lo, :] = xlo
                    XB[t][0, hi, :] = xhi
                    s2[0] = xlo * xlo if s2[0] is None else s2[0] + xlo * xlo
                    s2[1] = xhi * xhi if s2[1] is None else s2[1] + xhi * xhi
                if rp % 2 == 1:
                    yield
            var = jnp.sum(s2[0] + s2[1], axis=0, keepdims=True) * (1.0 / D)
            r1 = jax.lax.rsqrt(var + EPS)
            r2 = jax.lax.rsqrt(var * r1 * r1 + EPS)
            rr = r1 * r2
            for i in range(D // 16):
                HB[t][0, 16 * i: 16 * i + 16, :] = (XB[t][z, 16 * i: 16 * i + 16, :] * rr).astype(BF16)
            yield

    def act(get, off, w, zi, dts=range(5)):
        z = zz(zi)
        for r0 in range(0, w, 128):
            r1 = min(r0 + 128, w)
            j = (off + r0) // 128
            for i in dts:
                parts = []
                for q in range(r0, r1, 32):
                    u = get(q, q + 32, i) + b1c[z, off + q: off + q + 32, :]
                    parts.append(_gelu(u))
                g = jnp.concatenate(parts, axis=0).astype(BF16).T
                GB[j][0, 64 * i: 64 * i + 64, 0: r1 - r0] = pltpu.bitcast(g, U32)
                yield

    def mm1_dot(off, w, zi):
        z = zz(zi)
        rhs = jnp.concatenate([ldb(HB[t], z) for t in range(NTT)], axis=1)
        u = jax.lax.dot_general(w1t[off: off + w, :], rhs, NT, preferred_element_type=F32)
        return lambda r0, r1, i: u[r0:r1, _tile(i)]

    def mm1_step(tiles, first, final=None):
        z = zz()
        lhs = jnp.concatenate([w1t[0:W1C, _tile(t)] for t in tiles], axis=1)
        for i in range(5):
            rhs = jnp.concatenate([ldb(HB[t], z, slice(64 * i, 64 * i + 64)) for t in tiles], axis=1)
            part = jax.lax.dot_general(lhs, rhs, NT, preferred_element_type=F32)
            if final is not None:
                final.append(ACC[i][z] + part)
            else:
                ACC[i][0] = part if first else ACC[i][z] + part
            yield

    def mm2(c, tiles, d0=0, d1=D):
        z = zz(c % 8)
        rs = slice(d0 // 2, d1 // 2)
        parts = [GB[j][z, rs, :] for j in range(NFT - 1)] + [GB[NFT - 1][z, rs, 0: F % 128]]
        y = _dot(jnp.concatenate([pltpu.bitcast(p, BF16) for p in parts], axis=1),
                 jnp.concatenate([w2[:, _tile(t)] for t in tiles], axis=1))
        return [XB[t][zz(2), d0:d1, :] + (y[:, _tile(i)] + (bias[2][:, _tile(t)] + mean[t]))
                for i, t in enumerate(tiles)]

    chain = itertools.chain
    P = _PAIRS
    d_tables()
    U[0][0, :, 72:80, :] = jnp.zeros((2, 8, S), F32)
    s_tables()

    pend_v, fv_done, fm_done = [], [], []
    for c, seg in enumerate(_XSEG):
        last = c == len(_XSEG) - 1
        for t in seg:
            x_copy(t).wait()
        if c == 0:
            z_copy.wait()
            zpool.extend(sc["zs"][0, i] for i in range(NZ))
        if last:
            for cp in small:
                cp.wait()
        ready = [b for b in range(3) if b not in fm_done and all(4 * a + b in fv_done for a in range(4))]
        fm_done += ready
        cand = pend_v + seg
        fv, pend_v = (cand, []) if last else (cand[:-1], cand[-1:])
        fv_done += fv
        xg = x_in(seg)

        def fv_gen(tiles, xg=xg):
            for t in tiles:
                while t not in x_done:
                    next(xg)
                yield from front_vpu([t])

        _weave((xg, 5 * len(seg)), (fv_gen(fv), 4 * len(fv) + 2),
               (chain(*[front_mxu(b) for b in ready]) if ready else None, 5), (w_extra() if last else None, 5))
    _weave((chain(*[front_mxu(b) for b in range(4) if b not in fm_done]), 5))

    for layer in range(2):
        lay[0] = layer
        if layer == 0:
            for gs in ((0, 1), (2, 3), (4,)):
                for r in gs:
                    for cp in w_copies[r]:
                        cp.wait()
                _weave((pass_f(gs), 8), (chain(*([w_t1(r) for r in gs] + [w_t2(r) for r in gs])), 24 * len(gs)))
        else:
            fence()
            _weave((pass_f((0, 1, 2, 3, 4)), 8))
        for g in range(5):
            _weave((pass_i(g), 8))
        _weave((chain(*[pass_b(g, [0]) for g in range(4)]), 8))
        if layer == 0:
            w1_copy(0).wait()
        else:
            fence()
        ball = lambda b: chain(*[pass_b(g, [b]) for g in range(5)])
        _weave((pass_b(4, [0]), 2))
        _weave((ball(1), 10), (back_vpu(P[0]), 10))
        _weave((ball(2), 10), (back_vpu(P[1]), 10))
        _weave((ball(3), 10), (back_vpu(P[2]), 10))
        _weave((mm1_step(P[0] + P[1], True), 5), (back_vpu(P[3] + P[4]), 20))
        _weave((mm1_step(P[2] + P[3], False), 5), (back_vpu(P[5] + P[6] + P[7]), 30))
        _weave((mm1_step(P[4] + P[5], False), 5))
        fin = []
        get_fin = lambda r0, r1, q, fin=fin: fin[q][r0:r1]
        last = mm1_step(P[6] + P[7], False, fin)
        if layer == 0:
            _weave((bias_prep(), NFT))
        for i in range(5):
            next(last)
            if i >= 1:
                _weave((act(get_fin, 0, W1C, 0, [i - 1]), 1))
        if layer == 0:
            for i in range(1, NW1):
                w1_copy(i).wait()
        pend = (get_fin, 0, W1C, 0, [4])
        off = W1C
        for i, w in enumerate(W1S):
            if layer == 0 and i == len(W1S) - 1:
                for cp in [w2_copy(j) for j in range(NW2)] + seps:
                    cp.wait()
            cur = (mm1_dot(off, w, i + 1), off, w, i + 1)
            _weave((act(*pend), 1))
            pend = cur
            off += w
        _weave((act(*pend), 1))
        chunks = [P[0] + P[1], P[2] + P[3], P[4] + P[5], P[6], P[7]]
        nch = len(chunks)
        if layer == 0:
            for c in range(nch + 1):
                if c < nch:
                    for t, v in zip(chunks[c], mm2(c, chunks[c])):
                        XA[t][0] = v
                lay[0] = 1
                if c == nch:
                    _weave((front_mxu(2), 5), (front_vpu(chunks[c - 1]), 8))
                    _weave((front_mxu(3), 5))
                elif c >= 1:
                    _weave((front_vpu(chunks[c - 1]), 8))
                    if c <= 2:
                        _weave((front_mxu(c - 1), 5))
                lay[0] = 0
        else:
            jobs = [(c, chunks[c], 0, D) for c in range(nch - 1)]
            jobs += [(nch - 1, chunks[-1], 0, DS), (nch, chunks[-1], DS, D)]
            prev = None
            for n, job in enumerate(jobs + [None]):
                cur = (job, mm2(*job)) if job is not None else None
                if prev is not None:
                    (_, tiles, d0, d1), vals = prev
                    for i, (t, v) in enumerate(zip(tiles, vals)):
                        xio[_tile(t), d0:d1] = v.astype(BF16).T
                        outs.append(o_copy(t, d0, d1, NTT + i if d0 else None))
                        outs[-1].start()
                    if n in (nch - 2, nch):
                        fence()
                prev = cur

    for cp in outs:
        cp.wait()


@jax.jit
def pallas_interleave_layers__spectral_gfnet__mixer_token_mlp__prompt_kernel(A_x, A_w_r, A_w_i, B_x, B_w1, B_b1, B_w2, B_b2):
    del B_x
    any_spec = pl.BlockSpec(memory_space=pl.ANY)
    return pl.pallas_call(
        _kernel,
        out_shape=jax.ShapeDtypeStruct((1, S, D), BF16),
        in_specs=[any_spec] * 7,
        out_specs=any_spec,
        scratch_shapes=jax.tree_util.tree_leaves(_scratch(), is_leaf=_is_leaf),
        compiler_params=pltpu.CompilerParams(vmem_limit_bytes=120 * 1024 * 1024, disable_semaphore_checks=True),
    )(A_x, A_w_r.T, A_w_i.T, B_w1.T, B_b1, B_w2, B_b2)
```
